```python
import os as _os
_os.environ.setdefault("JAX_PLATFORMS", "cpu")
import jax
import jax.numpy as jnp

def _softmax(x, axis=-1):
    return jax.nn.softmax(x, axis=axis)
def _gelu(x):
    return jax.nn.gelu(x, approximate=True)
def _silu(x):
    return jax.nn.silu(x)
def _sigmoid(x):
    return jax.nn.sigmoid(x)
def _layernorm(x, axis=-1, eps=1e-5):
    m = jnp.mean(x, axis=axis, keepdims=True)
    v = jnp.var(x, axis=axis, keepdims=True)
    return (x - m) / jnp.sqrt(v + eps)
def _scatter_add(tgt, idx, src, axis=0):
    return tgt.at[idx].add(src)
def _segment_sum(src, seg, n):
    return jax.ops.segment_sum(src, seg, n)
class _Rng:
    def __init__(self, key):
        self._k = key
    def _next(self):
        self._k, sub = jax.random.split(self._k)
        return sub
    def normal(self, shape):
        return jax.random.normal(self._next(), shape, dtype=jnp.bfloat16)
    def randint(self, lo, hi, shape):
        return jax.random.randint(self._next(), shape, lo, hi, dtype=jnp.int32)
    def uniform(self, shape, lo=0.0, hi=1.0):
        return jax.random.uniform(self._next(), shape, jnp.bfloat16, lo, hi)
    def permutation(self, n):
        return jax.random.permutation(self._next(), n)


kernel_name = 'interleave_layers__mha_block__mixer_s_mlp__prompt'

def setup_inputs():
    _rng = _Rng(jax.random.key(int.from_bytes(__import__("os").urandom(4), "little")))
    _w = (lambda a: (lambda t: t.astype(jnp.bfloat16) if jnp.issubdtype(t.dtype, jnp.floating) else t)(jnp.asarray(a)))
    def _A_setup():
        B, S, D, H = 1, 2048, 448, 16
        return {
            "x": _w((lambda *s: _rng.normal(s) * 0.05)(B, S, D)),
            "wqkv": _w((lambda *s: _rng.normal(s) * 0.05)(D, 3 * D)),
            "wo": _w((lambda *s: _rng.normal(s) * 0.05)(D, D)),
        }
    _A_in = _A_setup()

    def _B_setup():
        B, S, D, F = 1, 2048, 448, 1792
        return {
            "x":  _w((lambda *s: _rng.normal(s) * 0.05)(B, S, D)),
            "w1": _w((lambda *s: _rng.normal(s) * 0.8)(D, D) * (D ** -0.5)),
            "w2": _w((lambda *s: _rng.normal(s) * 0.8)(D, D) * (D ** -0.5)),
            "w3": _w((lambda *s: _rng.normal(s) * 0.8)(D, F) * (D ** -0.5)),
            "w4": _w((lambda *s: _rng.normal(s) * 0.8)(F, D) * (F ** -0.5)),
        }
    _B_in = _B_setup()

    return {
        "A_x": _A_in["x"],
        "A_wqkv": _A_in["wqkv"],
        "A_wo": _A_in["wo"],
        "B_x": _B_in["x"],
        "B_w1": _B_in["w1"],
        "B_w2": _B_in["w2"],
        "B_w3": _B_in["w3"],
        "B_w4": _B_in["w4"],
    }

def reference(A_x, A_wqkv, A_wo, B_x, B_w1, B_w2, B_w3, B_w4):
    def _A_ref(x, wqkv, wo):
        B, S, D = x.shape
        H = 16
        Dh = D // H
        qkv = (lambda x, *d: x.transpose(*d))((x @ wqkv).reshape(B, S, 3, H, Dh), 2, 0, 3, 1, 4)
        q, k, v = qkv[0], qkv[1], qkv[2]
        scores = jnp.einsum("bhqd,bhkd->bhqk", q, k) * (Dh ** -0.5)
        p = _softmax(scores, axis=-1)
        o = jnp.einsum("bhqk,bhkd->bhqd", p, v)
        return (lambda x, *d: x.transpose(*d))(o, 0, 2, 1, 3).reshape(B, S, D) @ wo

    def _B_ref(x, w1, w2, w3, w4):
        B, S, D = x.shape
        h = _gelu(_layernorm(x, axis=-1) @ w1)
        c = D // 4
        g0 = jnp.pad(h[:, :, 0*c:1*c], ((0, 0), (1, 0), (0, 0)))[:, :S, :]
        g1 = jnp.pad(h[:, :, 1*c:2*c], ((0, 0), (0, 1), (0, 0)))[:, 1:, :]
        g2 = jnp.pad(h[:, :, 2*c:3*c], ((0, 0), (2, 0), (0, 0)))[:, :S, :]
        g3 = jnp.pad(h[:, :, 3*c:   ], ((0, 0), (0, 2), (0, 0)))[:, 2:, :]
        hs = jnp.concatenate([g0, g1, g2, g3], axis=-1) @ w2
        x1 = x + hs
        h2 = _gelu(_layernorm(x1, axis=-1) @ w3) @ w4
        return x1 + h2

    x = A_x
    x = x + _A_ref(_layernorm(x, axis=-1), A_wqkv, A_wo)
    x = x + _B_ref(_layernorm(x, axis=-1), B_w1, B_w2, B_w3, B_w4)
    x = x + _A_ref(_layernorm(x, axis=-1), A_wqkv, A_wo)
    x = x + _B_ref(_layernorm(x, axis=-1), B_w1, B_w2, B_w3, B_w4)
    return x
```

```python
import functools

import jax
import jax.numpy as jnp
from jax import lax
from jax.experimental import pallas as pl
from jax.experimental.pallas import tpu as pltpu

S, D, H, DH, F = 2048, 448, 16, 28, 1792
T = 512
NB = S // T
HG = 4
NG = H // HG
GD = HG * DH
CK = 128
C4 = D // 4
HALO = 128
EPS = 1e-5
QSCALE = (DH ** -0.5) * 1.4426950408889634
F32, BF16 = jnp.float32, jnp.bfloat16


def _layernorm(x):
    mean = jnp.sum(x, axis=0, keepdims=True) * (1.0 / D)
    d = x - mean
    var = jnp.sum(d * d, axis=0, keepdims=True) * (1.0 / D)
    return d * lax.rsqrt(var + EPS)


def _gelu(x):
    c0 = 0.7978845608028654
    t = jnp.tanh(x * (c0 + (c0 * 0.044715) * (x * x)))
    hx = 0.5 * x
    return hx + hx * t


def _dot(a, b):
    return jnp.dot(a, b, preferred_element_type=F32)


def _kernel(x_hbm, wqkv_hbm, wo_hbm, w1_hbm, w2_hbm, w3_hbm, w4t_hbm, out_hbm,
            io_buf, wqkv_raw, wo_raw, w1_raw, w2_raw, w3_raw, w4t,
            wqkvt, wot, w1t, w2t, w3t,
            xs, ys, ub, qt, kk, vt, ot, hbuf, gbuf, s_a, s_b, m_a, m_b,
            in_sem, out_sem, *, cfg):

    def x_copy(j):
        return pltpu.make_async_copy(
            x_hbm.at[:, pl.ds(j * T, T)], io_buf.at[j], in_sem.at[j])

    w_copies = [
        pltpu.make_async_copy(src, dst, in_sem.at[NB + n])
        for n, (src, dst) in enumerate((
            (wqkv_hbm, wqkv_raw), (wo_hbm, wo_raw), (w1_hbm, w1_raw),
            (w2_hbm, w2_raw), (w3_hbm, w3_raw), (w4t_hbm, w4t)))]

    def out_copy(j):
        return pltpu.make_async_copy(
            io_buf.at[j], out_hbm.at[:, pl.ds(j * T, T)], out_sem.at[j])

    x_copy(0).start()
    w_copies[0].start()
    for j in range(1, NB):
        x_copy(j).start()
    for c in w_copies[1:]:
        c.start()

    def qk_chunks(item, s_dst, m_dst):
        qb, g = item // NG, item % NG
        for j in range(HG):
            lo, hi = j * DH, (j + 1) * DH
            a, b = lo // 16 * 16, -(-hi // 16) * 16
            q = pltpu.bitcast(qt[qb, g, a:b, :], jnp.uint32)
            row = lax.broadcasted_iota(jnp.int32, q.shape, 0) + a // 2
            q = jnp.where((row >= lo // 2) & (row < hi // 2), q, jnp.uint32(0))
            parts = [q]
            if a:
                parts.insert(0, jnp.zeros((a // 2, T), jnp.uint32))
            parts.append(jnp.zeros(((128 - b) // 2, T), jnp.uint32))
            qm = pltpu.bitcast(jnp.concatenate(parts, axis=0), BF16)
            m = None
            for c in range(S // CK):
                sl = slice(c * CK, (c + 1) * CK)
                s = _dot(kk[g, sl, :], qm)
                s_dst[j, sl, :] = s
                mc = jnp.max(s.reshape(CK // 8, 8, T), axis=0)
                m = mc if m is None else jnp.maximum(m, mc)
                if c == S // CK - 1:
                    m_dst[j] = jnp.max(m, axis=0, keepdims=True)
                yield

    def pv_chunks(item, s_src, m_src):
        qb, g = item // NG, item % NG
        for j in range(HG):
            m = m_src[j]
            acc = None
            for c in range(S // CK):
                sl = slice(c * CK, (c + 1) * CK)
                p = jnp.exp2(s_src[j, sl, :] - m).astype(BF16)
                a = _dot(vt[g, j, c], p)
                acc = a if acc is None else acc + a
                if c == S // CK - 1:
                    inv = 1.0 / acc[DH:DH + 1, :]
                    ot[qb, g, 32 * j:32 * (j + 1), :] = (acc * inv).astype(BF16)
                yield

    def run(*gens):
        gens = list(gens)
        while gens:
            for gen in list(gens):
                try:
                    next(gen)
                except StopIteration:
                    gens.remove(gen)

    def attention_loop():
        def body(i, carry):
            @pl.when(i % 2 == 0)
            def _():
                run(qk_chunks(i + 1, s_b, m_b), pv_chunks(i, s_a, m_a))

            @pl.when(i % 2 == 1)
            def _():
                run(qk_chunks(i + 1, s_a, m_a), pv_chunks(i, s_b, m_b))
            return carry
        lax.fori_loop(0, NB * NG - 1, body, 0)

    def load_x(j):
        x_copy(j).wait()
        x = io_buf[j].astype(F32)
        xs[j] = x
        ub[j] = _layernorm(x).astype(BF16)

    def qkv(j):
        y = ub[j]
        q = _dot(wqkvt[0:D, :], y) * QSCALE
        qt[j] = q.astype(BF16).reshape(NG, GD, T)
        kv = _dot(wqkvt[D:3 * D, :], y)
        for g in range(NG):
            kk[g, j * T:(j + 1) * T, :] = kv[g * GD:g * GD + 128, :].T.astype(BF16)
        row = lax.broadcasted_iota(jnp.int32, (32, T), 0)
        for h in range(H):
            lo = D + h * DH
            if h < H - 1:
                v = kv[lo:lo + 32, :]
            else:
                v = jnp.concatenate([kv[lo:lo + DH, :], jnp.zeros((4, T), F32)], axis=0)
            v = jnp.where(row == DH, 1.0, v).astype(BF16)
            for c in range(T // CK):
                vt[h // HG, h % HG, j * (T // CK) + c] = v[:, c * CK:(c + 1) * CK]

    def proj_o(j):
        x = xs[j] + _dot(wot[...], ot[j].reshape(H * 32, T))
        xs[j] = x
        y = _layernorm(x)
        ys[j] = y
        ub[j] = _layernorm(y).astype(BF16)

    def mix1(j):
        h = _gelu(_dot(w1t[...], ub[j]))
        hbuf[:, HALO + j * T:HALO + (j + 1) * T] = pltpu.bitcast(h.astype(BF16), jnp.uint32)

    def mix2(j):
        parts = []
        for g, shift in enumerate((1, -1, 2, -2)):
            t0 = HALO + j * T - shift
            parts.append(hbuf[g * C4 // 2:(g + 1) * C4 // 2, t0:t0 + T])
        hs = pltpu.bitcast(jnp.concatenate(parts, axis=0), BF16)
        x1 = ys[j] + _dot(w2t[...], hs)
        xs[j] = xs[j] + x1
        ub[j] = _layernorm(x1).astype(BF16)

    def mlp1(j):
        u = ub[j]
        for n in range(F // 256):
            sl = slice(n * 256, (n + 1) * 256)
            gbuf[j % 2, sl, :] = _gelu(_dot(w3t[sl, :], u)).astype(BF16)

    def mlp2(j, last):
        x = xs[j] + _dot(w4t[...], gbuf[j % 2])
        if last:
            io_buf[j] = x.astype(BF16)
            out_copy(j).start()
        else:
            xs[j] = x
            ub[j] = _layernorm(x).astype(BF16)

    load_x(0)
    w_copies[0].wait()
    wqkvt[...] = wqkv_raw[...].T
    qkv(0)
    for j in range(1, NB):
        load_x(j)
        qkv(j)

    for c in w_copies[1:]:
        c.wait()
    wo = wo_raw[...].astype(F32)
    zeros = jnp.zeros((32 - DH, D), F32)
    wo_pad = jnp.concatenate(
        [p for h in range(H) for p in (wo[h * DH:(h + 1) * DH, :], zeros)], axis=0)
    wot[...] = wo_pad.T.astype(BF16)
    w1t[...] = w1_raw[...].T
    w2t[...] = w2_raw[...].T
    w3t[...] = w3_raw[...].T
    hbuf[:, 0:HALO] = jnp.zeros((D // 2, HALO), jnp.uint32)
    hbuf[:, HALO + S:] = jnp.zeros((D // 2, HALO), jnp.uint32)
    run(qk_chunks(0, s_a, m_a))

    for layer in range(2):
        last = layer == 1
        attention_loop()
        run(pv_chunks(NB * NG - 1, s_b, m_b))
        proj_o(0)
        proj_o(1)
        mix1(0)
        proj_o(2)
        mix1(1)
        proj_o(3)
        mix1(2)
        mix2(0)
        mix1(3)
        mix2(1)
        mlp1(0)
        mix2(2)
        mlp2(0, last)
        mlp1(1)
        mix2(3)
        mlp2(1, last)
        mlp1(2)
        if not last:
            qkv(0)
        mlp2(2, last)
        mlp1(3)
        if not last:
            qkv(1)
        mlp2(3, last)
        if not last:
            qkv(2)
            qkv(3)
            run(qk_chunks(0, s_a, m_a))

    for j in range(NB):
        out_copy(j).wait()


def build(cfg=None):
    cfg = dict(cfg or {})
    vm = pltpu.VMEM
    scratch = [
        vm((NB, D, T), BF16),
        vm((D, 3 * D), BF16), vm((D, D), BF16), vm((D, D), BF16), vm((D, D), BF16),
        vm((D, F), BF16), vm((D, F), BF16),
        vm((3 * D, D), BF16), vm((D, H * 32), BF16), vm((D, D), BF16), vm((D, D), BF16),
        vm((F, D), BF16),
        vm((NB, D, T), F32),
        vm((NB, D, T), F32),
        vm((NB, D, T), BF16),
        vm((NB, NG, GD, T), BF16),
        vm((NG, S, 128), BF16),
        vm((NG, HG, S // CK, 32, CK), BF16),
        vm((NB, NG, HG * 32, T), BF16),
        vm((D // 2, S + 2 * HALO), jnp.uint32),
        vm((2, F, T), BF16),
        vm((HG, S, T), F32), vm((HG, S, T), F32),
        vm((HG, 1, T), F32), vm((HG, 1, T), F32),
        pltpu.SemaphoreType.DMA((NB + 6,)),
        pltpu.SemaphoreType.DMA((NB,)),
    ]
    hbm = pl.BlockSpec(memory_space=pl.ANY)
    call = pl.pallas_call(
        functools.partial(_kernel, cfg=cfg),
        in_specs=[hbm] * 7,
        out_specs=hbm,
        out_shape=jax.ShapeDtypeStruct((D, S), BF16),
        scratch_shapes=scratch,
        compiler_params=pltpu.CompilerParams(vmem_limit_bytes=100 * 2**20),
    )

    @jax.jit
    def fn(A_x, A_wqkv, A_wo, B_x, B_w1, B_w2, B_w3, B_w4):
        del B_x
        out = call(A_x[0].T, A_wqkv, A_wo, B_w1, B_w2, B_w3, B_w4.T)
        return out.T[None]

    return fn


_kernel_fn = build()


@jax.jit
def pallas_interleave_layers__mha_block__mixer_s_mlp__prompt_kernel(
    A_x, A_wqkv, A_wo, B_x, B_w1, B_w2, B_w3, B_w4,
):
    return _kernel_fn(A_x, A_wqkv, A_wo, B_x, B_w1, B_w2, B_w3, B_w4)
```

```python
import functools

import jax
import jax.numpy as jnp
from jax import lax
from jax.experimental import pallas as pl
from jax.experimental.pallas import tpu as pltpu

S, D, H, DH, F = 2048, 448, 16, 28, 1792
T = 512
NB = S // T
NT = T // 128
HT = T // 2
HD = D // 2
HF = F // 2
HG = 4
NG = H // HG
GD = HG * DH
HP = 32
CK = 128
C4 = D // 4
HALO = 128
NV = 256
RG = 16
CN = 64
EPS = 1e-5
QSCALE = (DH ** -0.5) * 1.4426950408889634
DEN_LO, DEN_HI = 2.0 ** -20, 2.0 ** 40
F32_MAX = 3.4028234e38
F32, BF16, U32 = jnp.float32, jnp.bfloat16, jnp.uint32


def _gelu(x):
    c0 = 0.7978845608028654
    t = jnp.tanh(x * (c0 + (c0 * 0.044715) * (x * x)))
    hx = 0.5 * x
    return hx + hx * t


def _dot(a, b):
    return jnp.dot(a, b, preferred_element_type=F32)


def _lanes(t):
    return slice(t * 128, (t + 1) * 128)


def _lhs_terms(a11, a12, a21, a22):
    return (a11 + a22, a21 + a22, a11, a22, a11 + a12, a21 - a11, a12 - a22)


def _rhs_terms(b11, b12, b21, b22):
    return (b11 + b22, b11, b12 - b22, b21 - b11, b22, b11 + b12, b21 + b22)


_PRODUCT_ORDER = (
    (0, ((0, 1), (3, 1))), (1, ((2, 1), (3, -1))), (3, ((0, 1), (2, 1))),
    (2, ((1, 1), (3, 1))), (4, ((0, -1), (1, 1))), (5, ((3, 1),)), (6, ((0, 1),)))


def _overlap(*streams):
    done = [0] * len(streams)
    live = list(range(len(streams)))
    while live:
        k = min(live, key=lambda i: (done[i] + 0.5) / streams[i][1])
        if next(streams[k][0], StopIteration) is StopIteration:
            live.remove(k)
        done[k] += 1


def _chain(*streams):
    def gen():
        for stream, _ in streams:
            yield from stream
    return gen(), sum(n for _, n in streams)


def _ahead(stream):
    return stream[0], stream[1] * 110 // 100


def _load_bf16(ref, lead, row0, rows):
    return pltpu.bitcast(ref.bitcast(U32)[(*lead, pl.ds(row0 // 2, rows // 2))], BF16)


def _kernel(x_hbm, wqkv_hbm, wo_hbm, w1_hbm, w2_hbm, w3_hbm, w4t_hbm, out_hbm,
            sink, kb_a, kb_b, p_a, p_b, flag, rb, xs, ys, gb,
            aqkv, ao, a1, a2, a3, a4, hbuf, ot, qt, qf, kk, kn, vt,
            io_buf, wqkv_raw, wo_raw, w1_raw, w2_raw, w3_raw, w4t_raw,
            in_sem, out_sem):
    def x_copy(j):
        return pltpu.make_async_copy(
            x_hbm.at[:, pl.ds(j * T, T)], io_buf.at[j], in_sem.at[j])

    def w_copy(n, src, dst, lo=0, hi=None):
        cols = pl.ds(lo, (hi or src.shape[1]) - lo)
        return pltpu.make_async_copy(
            src.at[:, cols], dst.at[pl.ds(0, D), cols], in_sem.at[NB + n])

    wv_copy = w_copy(0, wqkv_hbm, wqkv_raw, 2 * D)
    wqk_copy = w_copy(1, wqkv_hbm, wqkv_raw, 0, 2 * D)
    w_copies = [w_copy(2 + n, src, dst) for n, (src, dst) in enumerate((
        (wo_hbm, wo_raw), (w1_hbm, w1_raw), (w2_hbm, w2_raw),
        (w3_hbm, w3_raw), (w4t_hbm, w4t_raw)))]

    def out_copy(j):
        return pltpu.make_async_copy(
            io_buf.at[j], out_hbm.at[:, pl.ds(j * T, T)], out_sem.at[j])

    pace = {}

    def pace_begin():
        lane = lax.broadcasted_iota(jnp.int32, (8, 128), 1)
        pace["keep"] = lane < 128 + (flag[:, 0:128] > 0.0).astype(jnp.int32)
        pace["v"] = jnp.zeros((8, 128), F32)
        pace["due"] = []

    def pace_end():
        for v in pace["due"]:
            tap(v)
        sink[0:8] = pace["v"]

    def tap(v):
        pace["v"] = jnp.maximum(pace["v"], v[0:8, 0:128])

    def due(v):
        pace["due"].append(v[0:8, 0:128])
        if len(pace["due"]) > 1:
            tap(pace["due"].pop(0))

    def gate(v):
        head = jnp.where(pace["keep"], v[0:8, 0:128], pace["v"])
        if v.shape[1] > 128:
            head = jnp.concatenate([head, v[0:8, 128:]], axis=1)
        return head if v.shape[0] == 8 else jnp.concatenate([head, v[8:]], axis=0)

    def put_lhs(dst, row0, a11, a12, a21, a22):
        for i, term in enumerate(_lhs_terms(a11, a12, a21, a22)):
            for c in range(dst.shape[1]):
                dst[i, c, row0:row0 + term.shape[0], :] = term[:, _lanes(c)].astype(BF16)
        terms = _lhs_terms(a11, a12, a21, a22)
        both = jnp.maximum(terms[5], terms[6])
        both = jnp.max(both.reshape(-1, 8, both.shape[1]), axis=0)
        due(functools.reduce(jnp.maximum, [both[:, _lanes(c)] for c in range(dst.shape[1])]))

    def prep(dst, row0, load, col0, n):
        first, stop = col0 // 128, -(-(col0 + n) // 128)

        def gen():
            halves = []
            for half in range(2):
                tiles = []
                for tile in range(first, stop):
                    w = pltpu.bitcast(gate(pltpu.bitcast(load(half, tile), F32)), BF16)
                    tiles.append(w.T)
                    yield
                halves.append(jnp.concatenate(tiles, axis=0))
            left, right = halves
            lo = col0 - first * 128
            for r in range(0, n // 2, 32):
                up, down = slice(lo + r, lo + r + 32), slice(lo + n // 2 + r, lo + n // 2 + r + 32)
                blocks = [w.astype(F32) for w in (left[up], right[up], left[down], right[down])]
                put_lhs(dst, row0 + r, gate(blocks[0]), *blocks[1:])
                yield
        return gen(), 2 * (stop - first) + n // 64

    def rows_of(raw):
        def load(half, tile):
            w = raw[half * HD:(half + 1) * HD, tile * 128:min(tile * 128 + 128, raw.shape[1])]
            if w.shape[1] < 128:
                w = jnp.concatenate([w, jnp.zeros((HD, 128 - w.shape[1]), BF16)], axis=1)
            return jnp.concatenate([w, jnp.zeros((256 - HD, 128), BF16)], axis=0)
        return load

    def head_rows_of(raw):
        def load(half, tile):
            w = rows_of(raw)(half, tile).astype(F32)
            row = lax.broadcasted_iota(jnp.int32, (HP, 128), 0)
            return jnp.concatenate(
                [jnp.where(row < DH, w[i * DH:i * DH + HP], 0.0) for i in range(H // 2)],
                axis=0).astype(BF16)
        return load

    def prep_w4():
        def gen():
            for r in range(0, HD, 16):
                blocks = [w4t_raw[n * HD + r:n * HD + r + 16, k * HF:(k + 1) * HF].astype(F32)
                          for n in range(2) for k in range(2)]
                put_lhs(a4, r, gate(blocks[0]), *blocks[1:])
                yield
        return gen(), HD // 16

    def lhs_of(ref, row0, rows):
        return lambda i: jnp.concatenate(
            [_load_bf16(ref, (i, c), row0, rows) for c in range(ref.shape[1])], axis=1)

    def rhs_of(ref, j, k):
        def get(i):
            r = jnp.concatenate([_load_bf16(ref, (j, i, t), 0, k) for t in range(2)], axis=1)
            if k % 128:
                r = jnp.concatenate([r, jnp.zeros((-k % 128, HT), BF16)], axis=0)
            return r
        return get

    def put_rhs(dst, t, row0, b11, b12, b21, b22):
        terms = _rhs_terms(b11, b12, b21, b22)
        for i, term in enumerate(terms):
            dst[i, t, pl.ds(row0, term.shape[0]), :] = term.astype(BF16)
        both = jnp.maximum(terms[2], terms[3])
        due(jnp.max(both.reshape(-1, 8, 128), axis=0))

    def put_rhs_tiles(dst, t, first, second):
        n = first.shape[0] // 2
        put_rhs(dst, t, 0, first[:n], second[:n], first[n:], second[n:])

    quadrants = ((0, 0), (0, 1), (1, 0), (1, 1))

    def head_q(h, qb):
        return jnp.concatenate([_load_bf16(qt, (h, qb, t), 0, HP) for t in range(NT)], axis=1)

    def spread_keys(h, kb, mark):
        def gen():
            for d in range(DH):
                for k0 in range(0, NV, NV // 2):
                    wide = jnp.broadcast_to(kn[h, k0:k0 + NV // 2, d:d + 1], (NV // 2, 128))
                    kb[d, k0:k0 + NV // 2] = wide
                    mark(wide[-8:])
                    yield
        return gen(), 2 * DH

    def exp_scores(h, qb, kb, p_dst, nv=NV):
        def vpu_scores(partial, k0, t0, half):
            acc = partial.pop((k0, t0), [None, None])
            for d in range(half * DH // 2, (half + 1) * DH // 2):
                key = kb[d, k0:k0 + 16, :]
                for x in range(2):
                    term = key * qf[h, qb, d:d + 1, _lanes(t0 + x)]
                    acc[x] = term if acc[x] is None else acc[x] + term
            for x in range(2):
                if half:
                    p_dst[qb, t0 + x, k0:k0 + 16, :] = jnp.exp2(acc[x]).astype(BF16)
                tap(acc[x][0:8])
                tap(acc[x][8:16])
            if not half:
                partial[k0, t0] = acc

        groups = (S - nv) // 16
        pieces = [(k0, t0, half) for k0 in range(0, nv, 16) for t0 in range(0, NT, 2)
                  for half in range(2)]
        pieces_at = {}
        for n, piece in enumerate(pieces):
            pieces_at.setdefault(int((n + 0.5) * groups / len(pieces)), []).append(piece)

        def gen():
            q = head_q(h, qb)
            partial = {}
            chunks = S // CK
            for c in range(chunks):
                r0, r1 = groups * c // chunks, groups * (c + 1) // chunks
                s = _dot(_load_bf16(kk, (h,), nv + 16 * r0, 16 * (r1 - r0)), q)
                for r in range(r0, r1):
                    sr = s[16 * (r - r0):16 * (r - r0 + 1), :]
                    e = jnp.exp2(sr)
                    for t in range(NT):
                        p_dst[qb, t, nv + 16 * r:nv + 16 * (r + 1), :] = e[:, _lanes(t)].astype(BF16)
                    i = r % (2 * NT)
                    tap(sr[8 * (i // NT):8 * (i // NT + 1), _lanes(i % NT)])
                    for piece in pieces_at.get(r, ()):
                        vpu_scores(partial, *piece)
                yield
        return gen(), S // CK

    def check_block(qb, heads):
        def gen():
            low = high = total = None
            for h in heads:
                acc = gate(jnp.concatenate([ot[h, qb, t] for t in range(NT)], axis=1))
                tail = acc[24:32]
                low = tail if low is None else jnp.minimum(low, tail)
                high = tail if high is None else jnp.maximum(high, tail)
                part = (acc[0:8] + acc[8:16]) + (acc[16:24] + tail)
                total = part if total is None else total + part
                if h == heads[-1]:
                    is_den = lax.broadcasted_iota(jnp.int32, (8, T), 0) == DH - 24
                    ok = ~is_den | ((low >= DEN_LO) & (high <= DEN_HI))
                    flag[...] = jnp.where(ok & (jnp.abs(total) <= F32_MAX), flag[...], 1.0)
                due(total[:, T - 128:])
                yield
        return gen(), len(heads)

    def weighted_values(h, qb, p_src, paced=False):
        def gen():
            acc = None
            for c in range(S // CK):
                p = jnp.concatenate(
                    [_load_bf16(p_src, (qb, t), c * CK, CK) for t in range(NT)], axis=1)
                a = _dot(_load_bf16(vt, (h, c), 0, HP), p)
                if paced:
                    tap(a)
                acc = a if acc is None else acc + a
                if c == S // CK - 1:
                    for t in range(NT):
                        ot[h, qb, t] = acc[:, _lanes(t)]
                yield
        return gen(), S // CK

    def attention_with_max():
        def body(item, carry):
            h, qb, t = item // (NB * NT), item // NT % NB, item % NT
            q = qt[h, qb, t]

            def scores(c):
                return _dot(kk[h, pl.ds(pl.multiple_of(c * CK, CK), CK), :], q)

            def row_max(c, m):
                return jnp.maximum(m, jnp.max(scores(c), axis=0, keepdims=True))

            m = lax.fori_loop(0, S // CK, row_max, jnp.full((1, 128), -jnp.inf, F32))

            def values(c, acc):
                return acc + _dot(vt[h, c], jnp.exp2(scores(c) - m).astype(BF16))

            ot[h, qb, t] = lax.fori_loop(0, S // CK, values, jnp.zeros((HP, 128), F32))
            return carry
        lax.fori_loop(0, H * NB * NT, body, 0)

    def own_block(emit):
        pl.when(jnp.max(flag[0:1, 0:128]) >= 0.0)(emit)

    def attention(peeled):
        def step(i, kb_cur, p_dst, kb_next, p_src):
            pace_begin()
            _overlap(_chain(*(exp_scores(i + 1, qb, kb_cur, p_dst) for qb in range(NB))),
                     _chain(*(weighted_values(i, qb, p_src) for qb in range(NB))),
                     spread_keys(jnp.minimum(i + 2, H - 1), kb_next, tap))
            pace_end()

        def body(i, carry):
            pl.when(i % 2 == 0)(lambda: step(i, kb_b, p_b, kb_a, p_a))
            pl.when(i % 2 == 1)(lambda: step(i, kb_a, p_a, kb_b, p_b))
            return carry

        if peeled:
            own_block(lambda: step(0, kb_b, p_b, kb_a, p_a))
        lax.fori_loop(int(peeled), H - 1, body, 0)

        pace_begin()
        early, late = range(H - 1), range(H - 1, H)
        for qb in range(NB):
            values = weighted_values(H - 1, qb, p_b, paced=True)
            if qb:
                _overlap(values, _chain(check_block(qb - 1, late), heads_to_rhs(qb - 1)))
            else:
                _overlap(values, _chain(*(check_block(j, early) for j in range(NB))))
        _overlap(check_block(NB - 1, late))
        pace_end()

        @pl.when(jnp.max(flag[...]) > 0.0)
        def _():
            attention_with_max()

            def redo(n, carry):
                pace_begin()
                head_to_rhs(n // H, n % 2, n // 2 % (H // 2))
                return carry
            lax.fori_loop(0, (NB - 1) * H, redo, 0)

    def block_product(lhs, rhs, rows, finish):
        groups = range(0, rows, RG)
        acc = {}
        left = [4, 2, 2, 4]
        for i, targets in _PRODUCT_ORDER:
            m = _dot(lhs(i), rhs(i))
            for blk, _ in targets:
                left[blk] -= 1
            for r in groups:
                piece = m[r:r + RG]
                tap(piece)
                for blk, sign in targets:
                    if (blk, r) not in acc:
                        acc[blk, r] = piece
                    else:
                        acc[blk, r] = acc[blk, r] + piece if sign > 0 else acc[blk, r] - piece
                    if not left[blk]:
                        finish(blk, r, acc.pop((blk, r)))
                yield

    def product_steps(rows):
        return 7 * (rows // RG)

    def moments(load):
        total = None
        for n in range(8):
            part = jnp.sum(gate(load(n)).reshape(7, 8, 128), axis=0)
            total = part if total is None else total + part
            if n % 4 == 3:
                due(total)
                yield
        mean = jnp.sum(total, axis=0, keepdims=True) * (1.0 / D)
        total = None
        for n in range(8):
            d = gate(load(n)) - mean
            part = jnp.sum((d * d).reshape(7, 8, 128), axis=0)
            total = part if total is None else total + part
            if n % 2 == 1:
                due(total)
                yield
        var = jnp.sum(total, axis=0, keepdims=True) * (1.0 / D)
        return mean, lax.rsqrt(var + EPS)

    def tile_rows(ref, j, u):
        return lambda n: ref[j, 56 * n:56 * (n + 1), _lanes(u)]

    def norm_to_rhs_gen(src_ref, j):
        for t in range(2):
            stats = []
            for u in (t, t + 2):
                stats.append((yield from moments(tile_rows(src_ref, j, u))))
            for r in range(0, HD, 16):
                blocks = [
                    (gate(src_ref[j, fh * HD + r:fh * HD + r + 16, _lanes(t + 2 * th)])
                     - stats[th][0]) * stats[th][1] for fh, th in quadrants]
                put_rhs(rb.at[j], t, r, *blocks)
                yield

    def norm_to_rhs(src_ref, j):
        return norm_to_rhs_gen(src_ref, j), 2 * (12 + 14)

    def norm_twice(j):
        def gen():
            for u in range(NT):
                mean, rstd = yield from moments(tile_rows(xs, j, u))
                for n in range(8):
                    y = (gate(xs[j, 56 * n:56 * (n + 1), _lanes(u)]) - mean) * rstd
                    ys[j, 56 * n:56 * (n + 1), _lanes(u)] = y
                    if n % 4 == 3:
                        due(y)
                        yield
        return _chain((gen(), NT * 8), norm_to_rhs(ys, j))

    def load_x(j):
        def gen():
            for r in range(0, D, 64):
                xs[j, r:r + 64] = io_buf[j, r:r + 64].astype(F32)
                yield
        return _chain((gen(), D // 64), norm_to_rhs(xs, j))

    def qkv(j):
        rhs = rhs_of(rb, j, HD)
        row = lax.broadcasted_iota(jnp.int32, (HP, HT), 0)

        def put_q(h, th, q):
            q = jnp.where(row < DH, q * QSCALE, 0.0)
            qf[h, j, :, th * HT:(th + 1) * HT] = q
            for t in range(2):
                qt[h, j, 2 * th + t] = q[:, _lanes(t)].astype(BF16)

        def put_k(h, th, k):
            k = k.astype(BF16).T
            kk[h, j * T + th * HT:j * T + (th + 1) * HT, :] = k
            if j == 0 and th == 0:
                kn[h] = k[0:NV].astype(F32)

        def put_v(h, th, v):
            v = jnp.where(row < DH, v, (row == DH).astype(F32))
            for t in range(2):
                vt[h, j * NT + 2 * th + t] = v[:, _lanes(t)].astype(BF16)

        def by_head(put):
            pieces = {}

            def finish(blk, r, piece):
                fh, th = quadrants[blk]
                pieces.setdefault(blk, []).append(piece)
                if r + RG == HD:
                    pieces[blk].append(jnp.zeros((8, HT), F32))
                have = sum(p.shape[0] for p in pieces[blk])
                for i in range(H // 2):
                    if r < i * DH + HP <= have:
                        c = jnp.concatenate(pieces[blk], axis=0)
                        put(fh * (H // 2) + i, th, c[i * DH:i * DH + HP])
            return finish

        return [(block_product(lhs_of(aqkv, n * HD, HD), rhs, HD, by_head(put)),
                 product_steps(HD)) for n, put in ((2, put_v), (1, put_k), (0, put_q))]

    def head_to_rhs(j, t, i):
        blocks = [gate(ot[fh * (H // 2) + i, j, t + 2 * th]) for fh, th in quadrants]
        put_rhs(rb.at[j], t, i * HP if isinstance(i, int) else pl.multiple_of(i * HP, HP),
                *(acc * (1.0 / acc[24:32])[DH - 24:DH - 23] for acc in blocks))

    def heads_to_rhs(j):
        def gen():
            for t in range(2):
                for i in range(H // 2):
                    head_to_rhs(j, t, i)
                    yield
        return gen(), H

    def place(blk, r):
        fh, th = quadrants[blk]
        return slice(fh * HD + r, fh * HD + r + RG), slice(th * HT, (th + 1) * HT)

    def proj_o(j):
        def finish(blk, r, c):
            rows, cols = place(blk, r)
            xs[j, rows, cols] = xs[j, rows, cols] + c
        return block_product(lhs_of(ao, 0, HD), rhs_of(rb, j, 256), HD, finish), product_steps(HD)

    def mix1(j):
        def finish(blk, r, c):
            rows, cols = place(blk, r)
            hbuf[rows, HALO + j * T + cols.start:HALO + j * T + cols.stop] = _gelu(c)
        return block_product(lhs_of(a1, 0, HD), rhs_of(rb, j, HD), HD, finish), product_steps(HD)

    def shift_to_rhs(j):
        def shifted(row, u):
            t0 = HALO + j * T + u * 128 - (1, -1, 2, -2)[row // C4]
            return gate(hbuf[row:row + 16, t0:t0 + 128])

        def gen():
            for t in range(2):
                for r in range(0, HD, 16):
                    blocks = [shifted(fh * HD + r, t + 2 * th) for fh, th in quadrants]
                    put_rhs(rb.at[j], t, r, *blocks)
                    yield
        return gen(), 28

    def mix2(j):
        def finish(blk, r, c):
            rows, cols = place(blk, r)
            x1 = ys[j, rows, cols] + c
            ys[j, rows, cols] = x1
            xs[j, rows, cols] = xs[j, rows, cols] + x1
        return block_product(lhs_of(a2, 0, HD), rhs_of(rb, j, HD), HD, finish), product_steps(HD)

    def mlp1(j):
        def gen():
            ready = []

            def activate():
                n, r, blocks = ready.pop(0)
                blocks = [_gelu(c) for c in blocks]
                for t in range(2):
                    put_rhs(gb.at[j % 2], t, n * CN + r, *(c[:, _lanes(t)] for c in blocks))

            for n in range(HF // CN):
                got = {}

                def finish(blk, r, c, n=n, got=got):
                    got[blk, r] = c
                    if all((b, r) in got for b in range(4)):
                        ready.append((n, r, [got.pop((b, r)) for b in range(4)]))

                waiting = len(ready)
                for x, _ in enumerate(block_product(
                        lhs_of(a3, n * CN, CN), rhs_of(rb, j, HD), CN, finish)):
                    if waiting and x % 7 == 3:
                        activate()
                        waiting -= 1
                    yield
            while ready:
                activate()
        return gen(), product_steps(HF)

    def mlp2(j, last=False):
        def finish(blk, r, c):
            rows, cols = place(blk, r)
            x = xs[j, rows, cols] + c
            if last:
                io_buf[j, rows, cols] = x.astype(BF16)
            else:
                xs[j, rows, cols] = x

        def gen():
            yield from block_product(lhs_of(a4, 0, HD), rhs_of(gb, j % 2, HF), HD, finish)
            if last:
                out_copy(j).start()
        return gen(), product_steps(HD)

    def start_attention(nv, *extra):
        def emit():
            pace_begin()
            _overlap(_chain(*(exp_scores(0, qb, kb_a, p_a, nv) for qb in range(NB))),
                     spread_keys(1, kb_b, due), *(make() for make in extra))
            pace_end()
        pace_end()
        own_block(emit)

    def into_first_layer():
        x_copy(0).start()
        wv_copy.start()
        x_copy(1).start()
        flag[...] = jnp.zeros((8, T), F32)
        hbuf[:, 0:HALO] = jnp.zeros((D, HALO), F32)
        hbuf[:, HALO + S:] = jnp.zeros((D, HALO), F32)
        pace_begin()
        wq, wk, wv = (prep(aqkv, n * HD, rows_of(wqkv_raw), n * D, D) for n in range(3))
        v, k, q = zip(*(qkv(j) for j in range(NB)))
        x_copy(0).wait()
        wv_copy.wait()
        wqk_copy.start()
        _overlap(load_x(0), wv)
        x_copy(1).wait()
        x_copy(2).start()
        x_copy(3).start()
        _overlap(v[0], load_x(1))
        wqk_copy.wait()
        _overlap(v[1], _chain(wk, wq))
        x_copy(2).wait()
        x_copy(3).wait()
        for c in w_copies:
            c.start()
        _overlap(_chain(k[0], q[0]), load_x(2))
        _overlap(_chain(k[1], q[1]), load_x(3))
        _overlap(_chain(k[2], q[2], v[2]), spread_keys(0, kb_a, due))
        for c in w_copies:
            c.wait()
        _overlap(_chain(k[3], q[3], v[3]), _ahead(_chain(
            prep(ao, 0, head_rows_of(wo_raw), 0, D), prep(a1, 0, rows_of(w1_raw), 0, D),
            prep(a2, 0, rows_of(w2_raw), 0, D), prep_w4())))
        start_attention(160, lambda: _ahead(prep(a3, 0, rows_of(w3_raw), 0, F)))

    def after_attention(last):
        pace_begin()
        _overlap(proj_o(0), heads_to_rhs(3))
        _overlap(_chain(proj_o(1), proj_o(2), proj_o(3), mix1(0), mix1(1)),
                 _chain(norm_twice(0), norm_twice(1), norm_twice(2)))
        _overlap(mix1(2), shift_to_rhs(0))
        _overlap(mix2(0), shift_to_rhs(1))
        _overlap(mix2(1), norm_to_rhs(ys, 0))
        _overlap(mlp1(0), norm_twice(3))
        _overlap(mix1(3))
        _overlap(mlp2(0, last),
                 _chain(norm_to_rhs(ys, 1), shift_to_rhs(2), shift_to_rhs(3)))
        _overlap(mix2(2))
        _overlap(mlp1(1), norm_to_rhs(ys, 2))
        _overlap(mix2(3))

    def into_second_layer():
        v, k, q = zip(*(qkv(j) for j in range(NB)))
        _overlap(mlp2(1), _chain(norm_to_rhs(ys, 3), norm_to_rhs(xs, 0)))
        _overlap(mlp1(2))
        _overlap(_chain(k[0], q[0], v[0]), norm_to_rhs(xs, 1))
        _overlap(mlp2(2), spread_keys(0, kb_a, due))
        _overlap(mlp1(3))
        _overlap(_chain(k[1], q[1], v[1]), norm_to_rhs(xs, 2))
        _overlap(mlp2(3))
        _overlap(_chain(k[2], q[2], v[2]), norm_to_rhs(xs, 3))
        _overlap(_chain(k[3], q[3], v[3]))
        start_attention(192)

    def into_output():
        _overlap(mlp2(1, True), norm_to_rhs(ys, 3))
        _overlap(mlp1(2))
        _overlap(mlp1(3))
        _overlap(mlp2(2, True))
        _overlap(mlp2(3, True))
        pace_end()
        for j in range(NB):
            out_copy(j).wait()

    into_first_layer()
    attention(peeled=True)
    after_attention(last=False)
    into_second_layer()
    attention(peeled=False)
    after_attention(last=True)
    into_output()


@jax.jit
def pallas_interleave_layers__mha_block__mixer_s_mlp__prompt_kernel(
    A_x: jax.Array,
    A_wqkv: jax.Array,
    A_wo: jax.Array,
    B_x: jax.Array,
    B_w1: jax.Array,
    B_w2: jax.Array,
    B_w3: jax.Array,
    B_w4: jax.Array,
):
    del B_x
    vm = pltpu.VMEM
    scratch = [
        vm((32, 128), F32),
        vm((DH, NV, 128), F32),
        vm((DH, NV, 128), F32),
        vm((NB, NT, S, 128), BF16),
        vm((NB, NT, S, 128), BF16),
        vm((8, T), F32),
        vm((NB, 7, 2, 256, 128), BF16),
        vm((NB, D, T), F32),
        vm((NB, D, T), F32),
        vm((2, 7, 2, HF, 128), BF16),
        vm((7, 2, 768, 128), BF16),
        vm((7, 2, 256, 128), BF16),
        vm((7, 2, 256, 128), BF16),
        vm((7, 2, 256, 128), BF16),
        vm((7, 2, HF, 128), BF16),
        vm((7, HF // 128, 256, 128), BF16),
        vm((D, S + 2 * HALO), F32),
        vm((H, NB, NT, HP, 128), F32),
        vm((H, NB, NT, HP, 128), BF16),
        vm((H, NB, HP, T), F32),
        vm((H, S, HP), BF16),
        vm((H, NV, HP), F32),
        vm((H, S // CK, HP, CK), BF16),
        vm((NB, D, T), BF16),
        vm((512, 3 * D), BF16), vm((D, D), BF16), vm((D, D), BF16), vm((D, D), BF16),
        vm((512, F), BF16), vm((512, F), BF16),
        pltpu.SemaphoreType.DMA((NB + 7,)),
        pltpu.SemaphoreType.DMA((NB,)),
    ]
    hbm = pl.BlockSpec(memory_space=pl.ANY)
    out = pl.pallas_call(
        _kernel,
        in_specs=[hbm] * 7,
        out_specs=hbm,
        out_shape=jax.ShapeDtypeStruct((D, S), BF16),
        scratch_shapes=scratch,
        compiler_params=pltpu.CompilerParams(vmem_limit_bytes=120 * 2**20),
    )(A_x[0].T, A_wqkv, A_wo, B_w1, B_w2, B_w3, B_w4.T)
    return out.T[None]
```

```python
import functools

import jax
import jax.numpy as jnp
from jax import lax
from jax.experimental import pallas as pl
from jax.experimental.pallas import tpu as pltpu

S, D, H, DH, F = 2048, 448, 16, 28, 1792
T = 512
NB = S // T
NT = T // 128
HT = T // 2
HD = D // 2
HF = F // 2
HP = 32
CK = 128
C4 = D // 4
HALO = 128
NV = 256
RG = 16
CN = 64
EPS = 1e-5
QSCALE = (DH ** -0.5) * 1.4426950408889634
DEN_LO, DEN_HI = 2.0 ** -20, 2.0 ** 40
F32_MAX = 3.4028234e38
F32, BF16, U32 = jnp.float32, jnp.bfloat16, jnp.uint32


def _gelu(x):
    c0 = 0.7978845608028654
    t = jnp.tanh(x * (c0 + (c0 * 0.044715) * (x * x)))
    hx = 0.5 * x
    return hx + hx * t


def _dot(a, b):
    return jnp.dot(a, b, preferred_element_type=F32)


def _lanes(t):
    return slice(t * 128, (t + 1) * 128)


def _lhs_terms(a11, a12, a21, a22):
    return (a11 + a22, a21 + a22, a11, a22, a11 + a12, a21 - a11, a12 - a22)


def _rhs_terms(b11, b12, b21, b22):
    return (b11 + b22, b11, b12 - b22, b21 - b11, b22, b11 + b12, b21 + b22)


_PRODUCT_ORDER = (
    (0, ((0, 1), (3, 1))), (1, ((2, 1), (3, -1))), (3, ((0, 1), (2, 1))),
    (2, ((1, 1), (3, 1))), (4, ((0, -1), (1, 1))), (5, ((3, 1),)), (6, ((0, 1),)))


def _overlap(*streams):
    done = [0] * len(streams)
    live = list(range(len(streams)))
    while live:
        k = min(live, key=lambda i: (done[i] + 0.5) / streams[i][1])
        if next(streams[k][0], StopIteration) is StopIteration:
            live.remove(k)
        done[k] += 1


def _chain(*streams):
    def gen():
        for stream, _ in streams:
            yield from stream
    return gen(), sum(n for _, n in streams)


def _ahead(stream):
    return stream[0], stream[1] * 110 // 100


def _load_bf16(ref, lead, row0, rows):
    return pltpu.bitcast(ref.bitcast(U32)[(*lead, pl.ds(row0 // 2, rows // 2))], BF16)


def _kernel(x_hbm, wqkv_hbm, wo_hbm, w1_hbm, w2_hbm, w3_hbm, w4t_hbm, out_hbm,
            sink, kb_a, kb_b, p_a, p_b, flag, rb, xs, ys, gb,
            aqkv, ao, a1, a2, a3, a4, hbuf, ot, qt, qf, kk, kn, vt,
            io_buf, wqkv_raw, wo_raw, w1_raw, w2_raw, w3_raw, w4t_raw,
            one, in_sem, out_sem):
    def x_copy(j):
        return pltpu.make_async_copy(
            x_hbm.at[:, pl.ds(j * T, T)], io_buf.at[j], in_sem.at[j])

    def w_copy(n, src, dst, lo=0, hi=None):
        cols = pl.ds(lo, (hi or src.shape[1]) - lo)
        return pltpu.make_async_copy(
            src.at[:, cols], dst.at[pl.ds(0, D), cols], in_sem.at[NB + n])

    wv_copy = w_copy(0, wqkv_hbm, wqkv_raw, 2 * D)
    wqk_copy = w_copy(1, wqkv_hbm, wqkv_raw, 0, 2 * D)
    w_copies = [w_copy(2 + n, src, dst) for n, (src, dst) in enumerate((
        (wo_hbm, wo_raw), (w1_hbm, w1_raw), (w2_hbm, w2_raw),
        (w3_hbm, w3_raw), (w4t_hbm, w4t_raw)))]

    def out_copy(j):
        return pltpu.make_async_copy(
            io_buf.at[j], out_hbm.at[:, pl.ds(j * T, T)], out_sem.at[j])

    def out_part_copy(blk):
        rows, cols = pl.ds(blk // 2 * HD, HD), blk % 2 * HT
        return pltpu.make_async_copy(
            io_buf.at[NB - 1, rows, pl.ds(cols, HT)],
            out_hbm.at[rows, pl.ds((NB - 1) * T + cols, HT)], out_sem.at[NB - 1 + blk])

    pace = {}

    def pace_begin():
        lane = lax.broadcasted_iota(jnp.int32, (8, 128), 1)
        pace["keep"] = lane < 128 + (flag[:, 0:128] > 0.0).astype(jnp.int32)
        pace["v"] = jnp.zeros((8, 128), F32)
        pace["due"] = []

    def pace_end():
        for v in pace["due"]:
            tap(v)
        sink[0:8] = pace["v"]

    def tap(v):
        pace["v"] = jnp.maximum(pace["v"], v[0:8, 0:128])

    def due(v):
        pace["due"].append(v[0:8, 0:128])
        if len(pace["due"]) > 1:
            tap(pace["due"].pop(0))

    def gate(v):
        head = jnp.where(pace["keep"], v[0:8, 0:128], pace["v"])
        if v.shape[1] > 128:
            head = jnp.concatenate([head, v[0:8, 128:]], axis=1)
        return head if v.shape[0] == 8 else jnp.concatenate([head, v[8:]], axis=0)

    def put_lhs(dst, row0, a11, a12, a21, a22):
        for i, term in enumerate(_lhs_terms(a11, a12, a21, a22)):
            for c in range(dst.shape[1]):
                dst[i, c, row0:row0 + term.shape[0], :] = term[:, _lanes(c)].astype(BF16)
        terms = _lhs_terms(a11, a12, a21, a22)
        both = jnp.maximum(terms[5], terms[6])
        both = jnp.max(both.reshape(-1, 8, both.shape[1]), axis=0)
        due(functools.reduce(jnp.maximum, [both[:, _lanes(c)] for c in range(dst.shape[1])]))

    def prep(dst, row0, load, col0, n):
        first, stop = col0 // 128, -(-(col0 + n) // 128)

        def gen():
            halves = []
            for half in range(2):
                tiles = []
                for tile in range(first, stop):
                    w = pltpu.bitcast(gate(pltpu.bitcast(load(half, tile), F32)), BF16)
                    tiles.append(w.T)
                    yield
                halves.append(jnp.concatenate(tiles, axis=0))
            left, right = halves
            lo = col0 - first * 128
            for r in range(0, n // 2, 32):
                up, down = slice(lo + r, lo + r + 32), slice(lo + n // 2 + r, lo + n // 2 + r + 32)
                blocks = [w.astype(F32) for w in (left[up], right[up], left[down], right[down])]
                put_lhs(dst, row0 + r, gate(blocks[0]), *blocks[1:])
                yield
        return gen(), 2 * (stop - first) + n // 64

    def rows_of(raw):
        def load(half, tile):
            w = raw[half * HD:(half + 1) * HD, tile * 128:min(tile * 128 + 128, raw.shape[1])]
            if w.shape[1] < 128:
                w = jnp.concatenate([w, jnp.zeros((HD, 128 - w.shape[1]), BF16)], axis=1)
            return jnp.concatenate([w, jnp.zeros((256 - HD, 128), BF16)], axis=0)
        return load

    def head_rows_of(raw):
        def load(half, tile):
            w = rows_of(raw)(half, tile).astype(F32)
            row = lax.broadcasted_iota(jnp.int32, (HP, 128), 0)
            return jnp.concatenate(
                [jnp.where(row < DH, w[i * DH:i * DH + HP], 0.0) for i in range(H // 2)],
                axis=0).astype(BF16)
        return load

    def prep_w4():
        def gen():
            for r in range(0, HD, 16):
                blocks = [w4t_raw[n * HD + r:n * HD + r + 16, k * HF:(k + 1) * HF].astype(F32)
                          for n in range(2) for k in range(2)]
                put_lhs(a4, r, gate(blocks[0]), *blocks[1:])
                yield
        return gen(), HD // 16

    def lhs_of(ref, row0, rows):
        return lambda i: jnp.concatenate(
            [_load_bf16(ref, (i, c), row0, rows) for c in range(ref.shape[1])], axis=1)

    def rhs_of(ref, j, k):
        def get(i):
            r = jnp.concatenate([_load_bf16(ref, (j, i, t), 0, k) for t in range(2)], axis=1)
            if k % 128:
                r = jnp.concatenate([r, jnp.zeros((-k % 128, HT), BF16)], axis=0)
            return r
        return get

    def put_rhs(dst, t, row0, b11, b12, b21, b22):
        terms = _rhs_terms(b11, b12, b21, b22)
        for i, term in enumerate(terms):
            dst[i, t, pl.ds(row0, term.shape[0]), :] = term.astype(BF16)
        both = jnp.maximum(terms[2], terms[3])
        due(jnp.max(both.reshape(-1, 8, 128), axis=0))

    quadrants = ((0, 0), (0, 1), (1, 0), (1, 1))

    def head_q(h, qb):
        return jnp.concatenate([_load_bf16(qt, (h, qb, t), 0, HP) for t in range(NT)], axis=1)

    def spread_keys(h, kb, mark):
        def gen():
            for d in range(DH):
                for k0 in range(0, NV, NV // 2):
                    wide = jnp.broadcast_to(kn[h, k0:k0 + NV // 2, d:d + 1], (NV // 2, 128))
                    kb[d, k0:k0 + NV // 2] = wide
                    mark(wide[-8:])
                    yield
        return gen(), 2 * DH

    def exp_scores(h, qb, kb, p_dst, nv=NV):
        def vpu_scores(partial, k0, t0, half):
            acc = partial.pop((k0, t0), [None, None])
            for d in range(half * DH // 2, (half + 1) * DH // 2):
                key = kb[d, k0:k0 + 16, :]
                for x in range(2):
                    term = key * qf[h, qb, d:d + 1, _lanes(t0 + x)]
                    acc[x] = term if acc[x] is None else acc[x] + term
            for x in range(2):
                if half:
                    p_dst[qb, t0 + x, k0:k0 + 16, :] = jnp.exp2(acc[x]).astype(BF16)
                tap(acc[x][0:8])
                tap(acc[x][8:16])
            if not half:
                partial[k0, t0] = acc

        groups = (S - nv) // 16
        pieces = [(k0, t0, half) for k0 in range(0, nv, 16) for t0 in range(0, NT, 2)
                  for half in range(2)]
        pieces_at = {}
        for n, piece in enumerate(pieces):
            pieces_at.setdefault(int((n + 0.5) * groups / len(pieces)), []).append(piece)

        def gen():
            q = head_q(h, qb)
            partial = {}
            chunks = S // CK
            for c in range(chunks):
                r0, r1 = groups * c // chunks, groups * (c + 1) // chunks
                s = _dot(_load_bf16(kk, (h,), nv + 16 * r0, 16 * (r1 - r0)), q)
                for r in range(r0, r1):
                    sr = s[16 * (r - r0):16 * (r - r0 + 1), :]
                    e = jnp.exp2(sr)
                    for t in range(NT):
                        p_dst[qb, t, nv + 16 * r:nv + 16 * (r + 1), :] = e[:, _lanes(t)].astype(BF16)
                    i = r % (2 * NT)
                    tap(sr[8 * (i // NT):8 * (i // NT + 1), _lanes(i % NT)])
                    for piece in pieces_at.get(r, ()):
                        vpu_scores(partial, *piece)
                yield
        return gen(), S // CK

    def check_block(qb, heads):
        def gen():
            low = high = total = None
            for h in heads:
                acc = gate(jnp.concatenate([ot[h, qb, t] for t in range(NT)], axis=1))
                tail = acc[24:32]
                low = tail if low is None else jnp.minimum(low, tail)
                high = tail if high is None else jnp.maximum(high, tail)
                part = (acc[0:8] + acc[8:16]) + (acc[16:24] + tail)
                total = part if total is None else total + part
                if h == heads[-1]:
                    is_den = lax.broadcasted_iota(jnp.int32, (8, T), 0) == DH - 24
                    ok = ~is_den | ((low >= DEN_LO) & (high <= DEN_HI))
                    flag[...] = jnp.where(ok & (jnp.abs(total) <= F32_MAX), flag[...], 1.0)
                due(total[:, T - 128:])
                yield
        return gen(), len(heads)

    def weighted_values(h, qb, p_src, paced=False):
        def gen():
            acc = None
            for c in range(S // CK):
                p = jnp.concatenate(
                    [_load_bf16(p_src, (qb, t), c * CK, CK) for t in range(NT)], axis=1)
                a = _dot(_load_bf16(vt, (h, c), 0, HP), p)
                if paced:
                    tap(a)
                acc = a if acc is None else acc + a
                if c == S // CK - 1:
                    for t in range(NT):
                        ot[h, qb, t] = acc[:, _lanes(t)]
                yield
        return gen(), S // CK

    def attention_with_max():
        def body(item, carry):
            h, qb, t = item // (NB * NT), item // NT % NB, item % NT
            q = qt[h, qb, t]

            def scores(c):
                return _dot(kk[h, pl.ds(pl.multiple_of(c * CK, CK), CK), :], q)

            def row_max(c, m):
                return jnp.maximum(m, jnp.max(scores(c), axis=0, keepdims=True))

            m = lax.fori_loop(0, S // CK, row_max, jnp.full((1, 128), -jnp.inf, F32))

            def values(c, acc):
                return acc + _dot(vt[h, c], jnp.exp2(scores(c) - m).astype(BF16))

            ot[h, qb, t] = lax.fori_loop(0, S // CK, values, jnp.zeros((HP, 128), F32))
            return carry
        lax.fori_loop(0, H * NB * NT, body, 0)

    def own_block(emit):
        pl.when(one[0] == 1)(emit)

    def attention(peeled):
        def step(i, kb_cur, p_dst, kb_next, p_src):
            pace_begin()
            _overlap(_chain(*(exp_scores(i + 1, qb, kb_cur, p_dst) for qb in range(NB))),
                     _chain(*(weighted_values(i, qb, p_src) for qb in range(NB))),
                     spread_keys(jnp.minimum(i + 2, H - 1), kb_next, tap))
            pace_end()

        def body(i, carry):
            pl.when(i % 2 == 0)(lambda: step(i, kb_b, p_b, kb_a, p_a))
            pl.when(i % 2 == 1)(lambda: step(i, kb_a, p_a, kb_b, p_b))
            return carry

        if peeled:
            own_block(lambda: step(0, kb_b, p_b, kb_a, p_a))
        lax.fori_loop(int(peeled), H - 1, body, 0)

        pace_begin()
        early, late = range(H - 1), range(H - 1, H)
        for qb in range(NB):
            values = weighted_values(H - 1, qb, p_b, paced=True)
            if qb:
                _overlap(values, _chain(check_block(qb - 1, late), heads_to_rhs(qb - 1)))
            else:
                _overlap(values, _chain(*(check_block(j, early) for j in range(NB))))
        _overlap(check_block(NB - 1, late))
        pace_end()

        @pl.when(jnp.max(flag[...]) > 0.0)
        def _():
            attention_with_max()

            def redo(n, carry):
                pace_begin()
                head_to_rhs(n // H, n % 2, n // 2 % (H // 2))
                return carry
            lax.fori_loop(0, (NB - 1) * H, redo, 0)

    def block_product(lhs, rhs, rows, finish):
        groups = range(0, rows, RG)
        acc = {}
        left = [4, 2, 2, 4]
        for i, targets in _PRODUCT_ORDER:
            m = _dot(lhs(i), rhs(i))
            for blk, _ in targets:
                left[blk] -= 1
            for r in groups:
                piece = m[r:r + RG]
                tap(piece)
                for blk, sign in targets:
                    if (blk, r) not in acc:
                        acc[blk, r] = piece
                    else:
                        acc[blk, r] = acc[blk, r] + piece if sign > 0 else acc[blk, r] - piece
                    if not left[blk]:
                        finish(blk, r, acc.pop((blk, r)))
                yield

    def product_steps(rows):
        return 7 * (rows // RG)

    def moments(load, twice=False):
        total = None
        for n in range(8):
            x = gate(load(n)) if n % 4 == 0 else load(n)
            part = jnp.sum(x.reshape(7, 8, 128), axis=0)
            total = part if total is None else total + part
            if n % 4 == 3:
                due(total)
                yield
        mean = jnp.sum(total, axis=0, keepdims=True) * (1.0 / D)
        squares = total = None
        for n in range(8):
            x = gate(load(n)) if n % 2 == 0 else load(n)
            d = (x - mean).reshape(7, 8, 128)
            part = jnp.sum(d * d, axis=0)
            squares = part if squares is None else squares + part
            if twice:
                part = jnp.sum(d, axis=0)
                total = part if total is None else total + part
            if n % 2 == 1:
                due(squares + total if twice else squares)
                yield
        var = jnp.sum(squares, axis=0, keepdims=True) * (1.0 / D)
        rstd = lax.rsqrt(var + EPS)
        if not twice:
            return mean, rstd
        mean_y = jnp.sum(total, axis=0, keepdims=True) * (1.0 / D) * rstd
        var_y = var * rstd * rstd - mean_y * mean_y
        return mean, rstd, mean_y, lax.rsqrt(var_y + EPS)

    def tile_rows(ref, j, u):
        return lambda n: ref[j, 56 * n:56 * (n + 1), _lanes(u)]

    def norm_to_rhs_gen(src_ref, j):
        for t in range(2):
            stats = []
            for u in (t, t + 2):
                stats.append((yield from moments(tile_rows(src_ref, j, u))))
            for r in range(0, HD, 16):
                blocks = [
                    (gate(src_ref[j, fh * HD + r:fh * HD + r + 16, _lanes(t + 2 * th)])
                     - stats[th][0]) * stats[th][1] for fh, th in quadrants]
                put_rhs(rb.at[j], t, r, *blocks)
                yield

    def norm_to_rhs(src_ref, j):
        return norm_to_rhs_gen(src_ref, j), 2 * (12 + 14)

    def norm_twice(j):
        def gen():
            for t in range(2):
                stats = []
                for u in (t, t + 2):
                    stats.append((yield from moments(tile_rows(xs, j, u), twice=True)))
                for r in range(0, HD, 16):
                    blocks = []
                    for fh, th in quadrants:
                        mean, rstd, mean_y, rstd_y = stats[th]
                        where = (j, slice(fh * HD + r, fh * HD + r + 16), _lanes(t + 2 * th))
                        y = (gate(xs[where]) - mean) * rstd
                        ys[where] = y
                        blocks.append((y - mean_y) * rstd_y)
                    put_rhs(rb.at[j], t, r, *blocks)
                    yield
        return gen(), 2 * (12 + 14)

    def load_x(j):
        def gen():
            for r in range(0, D, 64):
                xs[j, r:r + 64] = io_buf[j, r:r + 64].astype(F32)
                yield
        return _chain((gen(), D // 64), norm_to_rhs(xs, j))

    def qkv(j):
        rhs = rhs_of(rb, j, HD)
        row = lax.broadcasted_iota(jnp.int32, (HP, HT), 0)

        def put_q(h, th, q):
            q = jnp.where(row < DH, q * QSCALE, 0.0)
            qf[h, j, :, th * HT:(th + 1) * HT] = q
            for t in range(2):
                qt[h, j, 2 * th + t] = q[:, _lanes(t)].astype(BF16)

        def put_k(h, th, k):
            k = k.astype(BF16).T
            kk[h, j * T + th * HT:j * T + (th + 1) * HT, :] = k
            if j == 0 and th == 0:
                kn[h] = k[0:NV].astype(F32)

        def put_v(h, th, v):
            v = jnp.where(row < DH, v, (row == DH).astype(F32))
            for t in range(2):
                vt[h, j * NT + 2 * th + t] = v[:, _lanes(t)].astype(BF16)

        def by_head(put):
            pieces = {}

            def finish(blk, r, piece):
                fh, th = quadrants[blk]
                pieces.setdefault(blk, []).append(piece)
                if r + RG == HD:
                    pieces[blk].append(jnp.zeros((8, HT), F32))
                have = sum(p.shape[0] for p in pieces[blk])
                for i in range(H // 2):
                    if r < i * DH + HP <= have:
                        c = jnp.concatenate(pieces[blk], axis=0)
                        put(fh * (H // 2) + i, th, c[i * DH:i * DH + HP])
            return finish

        return [(block_product(lhs_of(aqkv, n * HD, HD), rhs, HD, by_head(put)),
                 product_steps(HD)) for n, put in ((2, put_v), (1, put_k), (0, put_q))]

    def head_to_rhs(j, t, i):
        blocks = [gate(ot[fh * (H // 2) + i, j, t + 2 * th]) for fh, th in quadrants]
        put_rhs(rb.at[j], t, i * HP if isinstance(i, int) else pl.multiple_of(i * HP, HP),
                *(acc * (1.0 / acc[24:32])[DH - 24:DH - 23] for acc in blocks))

    def heads_to_rhs(j):
        def gen():
            for t in range(2):
                for i in range(H // 2):
                    head_to_rhs(j, t, i)
                    yield
        return gen(), H

    def place(blk, r):
        fh, th = quadrants[blk]
        return slice(fh * HD + r, fh * HD + r + RG), slice(th * HT, (th + 1) * HT)

    def proj_o(j):
        def finish(blk, r, c):
            rows, cols = place(blk, r)
            xs[j, rows, cols] = xs[j, rows, cols] + c
        return block_product(lhs_of(ao, 0, HD), rhs_of(rb, j, 256), HD, finish), product_steps(HD)

    def mix1(j):
        def finish(blk, r, c):
            rows, cols = place(blk, r)
            hbuf[rows, HALO + j * T + cols.start:HALO + j * T + cols.stop] = _gelu(c)
        return block_product(lhs_of(a1, 0, HD), rhs_of(rb, j, HD), HD, finish), product_steps(HD)

    def shift_to_rhs(j):
        def shifted(row, u):
            t0 = HALO + j * T + u * 128 - (1, -1, 2, -2)[row // C4]
            return gate(hbuf[row:row + 16, t0:t0 + 128])

        def gen():
            for t in range(2):
                for r in range(0, HD, 16):
                    blocks = [shifted(fh * HD + r, t + 2 * th) for fh, th in quadrants]
                    put_rhs(rb.at[j], t, r, *blocks)
                    yield
        return gen(), 28

    def mix2(j):
        def finish(blk, r, c):
            rows, cols = place(blk, r)
            x1 = ys[j, rows, cols] + c
            ys[j, rows, cols] = x1
            xs[j, rows, cols] = xs[j, rows, cols] + x1
        return block_product(lhs_of(a2, 0, HD), rhs_of(rb, j, HD), HD, finish), product_steps(HD)

    def mlp1(j):
        def gen():
            ready = []

            def activate():
                n, r, blocks = ready.pop(0)
                blocks = [_gelu(c) for c in blocks]
                for t in range(2):
                    put_rhs(gb.at[j % 2], t, n * CN + r, *(c[:, _lanes(t)] for c in blocks))

            for n in range(HF // CN):
                got = {}

                def finish(blk, r, c, n=n, got=got):
                    got[blk, r] = c
                    if all((b, r) in got for b in range(4)):
                        ready.append((n, r, [got.pop((b, r)) for b in range(4)]))

                waiting = len(ready)
                for x, _ in enumerate(block_product(
                        lhs_of(a3, n * CN, CN), rhs_of(rb, j, HD), CN, finish)):
                    if waiting and x % 7 == 3:
                        activate()
                        waiting -= 1
                    yield
            while ready:
                activate()
        return gen(), product_steps(HF)

    def mlp2(j, last=False):
        def finish(blk, r, c):
            rows, cols = place(blk, r)
            x = xs[j, rows, cols] + c
            if last:
                io_buf[j, rows, cols] = x.astype(BF16)
                if j == NB - 1 and r + RG == HD:
                    out_part_copy(blk).start()
            else:
                xs[j, rows, cols] = x

        def gen():
            yield from block_product(lhs_of(a4, 0, HD), rhs_of(gb, j % 2, HF), HD, finish)
            if last and j < NB - 1:
                out_copy(j).start()
        return gen(), product_steps(HD)

    def start_attention(nv, *extra):
        def emit():
            pace_begin()
            _overlap(_chain(*(exp_scores(0, qb, kb_a, p_a, nv) for qb in range(NB))),
                     spread_keys(1, kb_b, due), *(make() for make in extra))
            pace_end()
        pace_end()
        own_block(emit)

    def into_first_layer():
        x_copy(0).start()
        wv_copy.start()
        x_copy(1).start()
        flag[...] = jnp.zeros((8, T), F32)
        one[0] = 1
        hbuf[:, 0:HALO] = jnp.zeros((D, HALO), F32)
        hbuf[:, HALO + S:] = jnp.zeros((D, HALO), F32)
        pace_begin()
        wq, wk, wv = (prep(aqkv, n * HD, rows_of(wqkv_raw), n * D, D) for n in range(3))
        v, k, q = zip(*(qkv(j) for j in range(NB)))
        x_copy(0).wait()
        wv_copy.wait()
        wqk_copy.start()
        _overlap(load_x(0), wv)
        x_copy(1).wait()
        x_copy(2).start()
        x_copy(3).start()
        _overlap(v[0], load_x(1))
        wqk_copy.wait()
        _overlap(v[1], _chain(wk, wq))
        x_copy(2).wait()
        x_copy(3).wait()
        for c in w_copies:
            c.start()
        _overlap(_chain(k[0], q[0]), load_x(2))
        _overlap(_chain(k[1], q[1]), load_x(3))
        _overlap(_chain(k[2], q[2], v[2]), spread_keys(0, kb_a, due))
        for c in w_copies:
            c.wait()
        _overlap(_chain(k[3], q[3], v[3]), _ahead(_chain(
            prep(ao, 0, head_rows_of(wo_raw), 0, D), prep(a1, 0, rows_of(w1_raw), 0, D),
            prep(a2, 0, rows_of(w2_raw), 0, D), prep_w4())))
        start_attention(160, lambda: _ahead(prep(a3, 0, rows_of(w3_raw), 0, F)))

    def after_attention(last):
        pace_begin()
        _overlap(proj_o(0), heads_to_rhs(3))
        _overlap(_chain(proj_o(1), proj_o(2), proj_o(3), mix1(0), mix1(1)),
                 _chain(norm_twice(0), norm_twice(1), norm_twice(2), norm_twice(3)))
        _overlap(mix1(2), shift_to_rhs(0))
        _overlap(mix2(0), shift_to_rhs(1))
        _overlap(mix2(1), norm_to_rhs(ys, 0))
        _overlap(mix1(3))
        _overlap(mlp1(0), _chain(norm_to_rhs(ys, 1), shift_to_rhs(2), shift_to_rhs(3)))
        _overlap(mlp2(0, last))
        _overlap(mix2(2))
        _overlap(mlp1(1), norm_to_rhs(ys, 2))
        _overlap(mix2(3))

    def into_second_layer():
        v, k, q = zip(*(qkv(j) for j in range(NB)))
        _overlap(mlp2(1), _chain(norm_to_rhs(ys, 3), norm_to_rhs(xs, 0)))
        _overlap(mlp1(2))
        _overlap(_chain(k[0], q[0], v[0]), norm_to_rhs(xs, 1))
        _overlap(mlp2(2), spread_keys(0, kb_a, due))
        _overlap(mlp1(3))
        _overlap(_chain(k[1], q[1], v[1]), norm_to_rhs(xs, 2))
        _overlap(mlp2(3))
        _overlap(_chain(k[2], q[2], v[2]), norm_to_rhs(xs, 3))
        _overlap(_chain(k[3], q[3], v[3]))
        start_attention(192)

    def into_output():
        _overlap(mlp2(1, True), norm_to_rhs(ys, 3))
        _overlap(mlp1(2))
        _overlap(mlp1(3))
        _overlap(mlp2(2, True))
        _overlap(mlp2(3, True))
        pace_end()
        for j in range(NB - 1):
            out_copy(j).wait()
        for blk in range(4):
            out_part_copy(blk).wait()

    into_first_layer()
    attention(peeled=True)
    after_attention(last=False)
    into_second_layer()
    attention(peeled=False)
    after_attention(last=True)
    into_output()


@jax.jit
def pallas_interleave_layers__mha_block__mixer_s_mlp__prompt_kernel(
    A_x: jax.Array,
    A_wqkv: jax.Array,
    A_wo: jax.Array,
    B_x: jax.Array,
    B_w1: jax.Array,
    B_w2: jax.Array,
    B_w3: jax.Array,
    B_w4: jax.Array,
):
    del B_x
    vm = pltpu.VMEM
    scratch = [
        vm((32, 128), F32),
        vm((DH, NV, 128), F32),
        vm((DH, NV, 128), F32),
        vm((NB, NT, S, 128), BF16),
        vm((NB, NT, S, 128), BF16),
        vm((8, T), F32),
        vm((NB, 7, 2, 256, 128), BF16),
        vm((NB, D, T), F32),
        vm((NB, D, T), F32),
        vm((2, 7, 2, HF, 128), BF16),
        vm((7, 2, 768, 128), BF16),
        vm((7, 2, 256, 128), BF16),
        vm((7, 2, 256, 128), BF16),
        vm((7, 2, 256, 128), BF16),
        vm((7, 2, HF, 128), BF16),
        vm((7, HF // 128, 256, 128), BF16),
        vm((D, S + 2 * HALO), F32),
        vm((H, NB, NT, HP, 128), F32),
        vm((H, NB, NT, HP, 128), BF16),
        vm((H, NB, HP, T), F32),
        vm((H, S, HP), BF16),
        vm((H, NV, HP), F32),
        vm((H, S // CK, HP, CK), BF16),
        vm((NB, D, T), BF16),
        vm((512, 3 * D), BF16), vm((D, D), BF16), vm((D, D), BF16), vm((D, D), BF16),
        vm((512, F), BF16), vm((512, F), BF16),
        pltpu.SMEM((1,), jnp.int32),
        pltpu.SemaphoreType.DMA((NB + 7,)),
        pltpu.SemaphoreType.DMA((NB + 3,)),
    ]
    hbm = pl.BlockSpec(memory_space=pl.ANY)
    out = pl.pallas_call(
        _kernel,
        in_specs=[hbm] * 7,
        out_specs=hbm,
        out_shape=jax.ShapeDtypeStruct((D, S), BF16),
        scratch_shapes=scratch,
        compiler_params=pltpu.CompilerParams(vmem_limit_bytes=120 * 2**20),
    )(A_x[0].T, A_wqkv, A_wo, B_w1, B_w2, B_w3, B_w4.T)
    return out.T[None]
```

```python
import functools

import jax
import jax.numpy as jnp
from jax import lax
from jax.experimental import pallas as pl
from jax.experimental.pallas import tpu as pltpu

S, D, H, DH, F = 2048, 448, 16, 28, 1792
T = 512
NB = S // T
NT = T // 128
HT = T // 2
HD = D // 2
HF = F // 2
HP = 32
CK = 128
C4 = D // 4
HALO = 128
NV = 256
RG = 16
CN = 64
EPS = 1e-5
QSCALE = (DH ** -0.5) * 1.4426950408889634
DEN_LO, DEN_HI = 2.0 ** -20, 2.0 ** 40
F32_MAX = 3.4028234e38
F32, BF16, U32 = jnp.float32, jnp.bfloat16, jnp.uint32


def _gelu(x):
    c0 = 0.7978845608028654
    t = jnp.tanh(x * (c0 + (c0 * 0.044715) * (x * x)))
    hx = 0.5 * x
    return hx + hx * t


def _dot(a, b):
    return jnp.dot(a, b, preferred_element_type=F32)


def _lanes(t):
    return slice(t * 128, (t + 1) * 128)


def _lhs_terms(a11, a12, a21, a22):
    return (a11 + a22, a21 + a22, a11, a22, a11 + a12, a21 - a11, a12 - a22)


def _rhs_terms(b11, b12, b21, b22):
    return (b11 + b22, b11, b12 - b22, b21 - b11, b22, b11 + b12, b21 + b22)


_PRODUCT_ORDER = (
    (1, ((2, 1), (3, -1))), (3, ((0, 1), (2, 1))), (0, ((0, 1), (3, 1))), (6, ((0, 1),)),
    (4, ((0, -1), (1, 1))), (2, ((1, 1), (3, 1))), (5, ((3, 1),)))


def _overlap(*streams):
    done = [0] * len(streams)
    live = list(range(len(streams)))
    while live:
        k = min(live, key=lambda i: (done[i] + 0.5) / streams[i][1])
        if next(streams[k][0], StopIteration) is StopIteration:
            live.remove(k)
        done[k] += 1


def _chain(*streams):
    def gen():
        for stream, _ in streams:
            yield from stream
    return gen(), sum(n for _, n in streams)


def _ahead(stream):
    return stream[0], stream[1] * 110 // 100


def _load_bf16(ref, lead, row0, rows):
    return pltpu.bitcast(ref.bitcast(U32)[(*lead, pl.ds(row0 // 2, rows // 2))], BF16)


def _kernel(x_hbm, wqkv_hbm, wo_hbm, w1_hbm, w2_hbm, w3_hbm, w4t_hbm, out_hbm,
            sink, kb_a, kb_b, p_a, p_b, flag, rb, xs, ys, gb,
            aqkv, ao, a1, a2, a3, a4, hbuf, ot, qt, qf, kk, kn, vt,
            io_buf, wqkv_raw, wo_raw, w1_raw, w2_raw, w3_raw, w4t_raw,
            one, in_sem, out_sem):
    def x_copy(j):
        return pltpu.make_async_copy(
            x_hbm.at[:, pl.ds(j * T, T)], io_buf.at[j], in_sem.at[j])

    def w_copy(n, src, dst, lo=0, hi=None):
        cols = pl.ds(lo, (hi or src.shape[1]) - lo)
        return pltpu.make_async_copy(
            src.at[:, cols], dst.at[pl.ds(0, D), cols], in_sem.at[NB + n])

    wv_copy = w_copy(0, wqkv_hbm, wqkv_raw, 2 * D)
    wqk_copy = w_copy(1, wqkv_hbm, wqkv_raw, 0, 2 * D)
    w_copies = [w_copy(2 + n, src, dst) for n, (src, dst) in enumerate((
        (wo_hbm, wo_raw), (w1_hbm, w1_raw), (w2_hbm, w2_raw),
        (w3_hbm, w3_raw), (w4t_hbm, w4t_raw)))]

    def out_copy(j):
        return pltpu.make_async_copy(
            io_buf.at[j], out_hbm.at[:, pl.ds(j * T, T)], out_sem.at[j])

    def out_part_copy(blk):
        rows, cols = pl.ds(blk // 2 * HD, HD), blk % 2 * HT
        return pltpu.make_async_copy(
            io_buf.at[NB - 1, rows, pl.ds(cols, HT)],
            out_hbm.at[rows, pl.ds((NB - 1) * T + cols, HT)], out_sem.at[NB - 1 + blk])

    pace = {}

    def pace_begin():
        lane = lax.broadcasted_iota(jnp.int32, (8, 128), 1)
        pace["keep"] = lane < 128 + (flag[:, 0:128] > 0.0).astype(jnp.int32)
        pace["v"] = jnp.zeros((8, 128), F32)
        pace["due"] = []

    def pace_end():
        for v in pace["due"]:
            tap(v)
        sink[0:8] = pace["v"]

    def tap(v):
        pace["v"] = jnp.maximum(pace["v"], v[0:8, 0:128])

    def due(v):
        pace["due"].append(v[0:8, 0:128])
        if len(pace["due"]) > 1:
            tap(pace["due"].pop(0))

    def gate(v):
        head = jnp.where(pace["keep"], v[0:8, 0:128], pace["v"])
        if v.shape[1] > 128:
            head = jnp.concatenate([head, v[0:8, 128:]], axis=1)
        return head if v.shape[0] == 8 else jnp.concatenate([head, v[8:]], axis=0)

    def put_lhs(dst, row0, a11, a12, a21, a22):
        for i, term in enumerate(_lhs_terms(a11, a12, a21, a22)):
            for c in range(dst.shape[1]):
                dst[i, c, row0:row0 + term.shape[0], :] = term[:, _lanes(c)].astype(BF16)
        terms = _lhs_terms(a11, a12, a21, a22)
        both = jnp.maximum(terms[5], terms[6])
        both = jnp.max(both.reshape(-1, 8, both.shape[1]), axis=0)
        due(functools.reduce(jnp.maximum, [both[:, _lanes(c)] for c in range(dst.shape[1])]))

    def prep(dst, row0, load, col0, n):
        first, stop = col0 // 128, -(-(col0 + n) // 128)

        def gen():
            halves = []
            for half in range(2):
                tiles = []
                for tile in range(first, stop):
                    w = pltpu.bitcast(gate(pltpu.bitcast(load(half, tile), F32)), BF16)
                    tiles.append(w.T)
                    yield
                halves.append(jnp.concatenate(tiles, axis=0))
            left, right = halves
            lo = col0 - first * 128
            for r in range(0, n // 2, 32):
                up, down = slice(lo + r, lo + r + 32), slice(lo + n // 2 + r, lo + n // 2 + r + 32)
                blocks = [w.astype(F32) for w in (left[up], right[up], left[down], right[down])]
                put_lhs(dst, row0 + r, gate(blocks[0]), *blocks[1:])
                yield
        return gen(), 2 * (stop - first) + n // 64

    def rows_of(raw):
        def load(half, tile):
            w = raw[half * HD:(half + 1) * HD, tile * 128:min(tile * 128 + 128, raw.shape[1])]
            if w.shape[1] < 128:
                w = jnp.concatenate([w, jnp.zeros((HD, 128 - w.shape[1]), BF16)], axis=1)
            return jnp.concatenate([w, jnp.zeros((256 - HD, 128), BF16)], axis=0)
        return load

    def head_rows_of(raw):
        def load(half, tile):
            w = rows_of(raw)(half, tile).astype(F32)
            row = lax.broadcasted_iota(jnp.int32, (HP, 128), 0)
            return jnp.concatenate(
                [jnp.where(row < DH, w[i * DH:i * DH + HP], 0.0) for i in range(H // 2)],
                axis=0).astype(BF16)
        return load

    def prep_w4():
        def gen():
            for r in range(0, HD, 16):
                blocks = [w4t_raw[n * HD + r:n * HD + r + 16, k * HF:(k + 1) * HF].astype(F32)
                          for n in range(2) for k in range(2)]
                put_lhs(a4, r, gate(blocks[0]), *blocks[1:])
                yield
        return gen(), HD // 16

    def lhs_of(ref, row0, rows):
        return lambda i: jnp.concatenate(
            [_load_bf16(ref, (i, c), row0, rows) for c in range(ref.shape[1])], axis=1)

    def rhs_of(ref, j, k):
        def get(i):
            r = jnp.concatenate([_load_bf16(ref, (j, i, t), 0, k) for t in range(2)], axis=1)
            if k % 128:
                r = jnp.concatenate([r, jnp.zeros((-k % 128, HT), BF16)], axis=0)
            return r
        return get

    def put_rhs(dst, t, row0, b11, b12, b21, b22):
        terms = _rhs_terms(b11, b12, b21, b22)
        for i, term in enumerate(terms):
            dst[i, t, pl.ds(row0, term.shape[0]), :] = term.astype(BF16)
        both = jnp.maximum(terms[2], terms[3])
        due(jnp.max(both.reshape(-1, 8, 128), axis=0))

    quadrants = ((0, 0), (0, 1), (1, 0), (1, 1))

    def head_q(h, qb):
        return jnp.concatenate([_load_bf16(qt, (h, qb, t), 0, HP) for t in range(NT)], axis=1)

    def spread_keys(h, kb):
        n = NV // 4

        def gen():
            for d in range(DH):
                for k0 in range(0, NV, n):
                    wide = jnp.broadcast_to(kn[h, k0:k0 + n, d:d + 1], (n, 128))
                    kb[d, k0:k0 + n] = wide
                    due(wide[-8:])
                    yield
        return gen(), 4 * DH

    def exp_scores(h, qb, kb, p_dst, nv=NV):
        def vpu_scores(partial, k0, t0, half):
            acc = partial.pop((k0, t0), [None, None])
            for d in range(half * DH // 2, (half + 1) * DH // 2):
                key = kb[d, k0:k0 + 16, :]
                for x in range(2):
                    term = key * qf[h, qb, d:d + 1, _lanes(t0 + x)]
                    acc[x] = term if acc[x] is None else acc[x] + term
            for x in range(2):
                if half:
                    p_dst[qb, t0 + x, k0:k0 + 16, :] = jnp.exp2(acc[x]).astype(BF16)
                tap(acc[x][0:8])
                tap(acc[x][8:16])
            if not half:
                partial[k0, t0] = acc

        groups = (S - nv) // 16
        pieces = [(k0, t0, half) for k0 in range(0, nv, 16) for t0 in range(0, NT, 2)
                  for half in range(2)]
        pieces_at = {}
        for n, piece in enumerate(pieces):
            pieces_at.setdefault(int((n + 0.5) * groups / len(pieces)), []).append(piece)

        def gen():
            q = head_q(h, qb)
            partial = {}
            chunks = S // CK
            for c in range(chunks):
                r0, r1 = groups * c // chunks, groups * (c + 1) // chunks
                s = _dot(_load_bf16(kk, (h,), nv + 16 * r0, 16 * (r1 - r0)), q)
                for r in range(r0, r1):
                    sr = s[16 * (r - r0):16 * (r - r0 + 1), :]
                    e = jnp.exp2(sr)
                    for t in range(NT):
                        p_dst[qb, t, nv + 16 * r:nv + 16 * (r + 1), :] = e[:, _lanes(t)].astype(BF16)
                    i = r % (2 * NT)
                    tap(sr[8 * (i // NT):8 * (i // NT + 1), _lanes(i % NT)])
                    for piece in pieces_at.get(r, ()):
                        vpu_scores(partial, *piece)
                yield
        return gen(), S // CK

    def check_block(qb, heads):
        def gen():
            low = high = total = None
            for h in heads:
                acc = gate(jnp.concatenate([ot[h, qb, t] for t in range(NT)], axis=1))
                tail = acc[24:32]
                low = tail if low is None else jnp.minimum(low, tail)
                high = tail if high is None else jnp.maximum(high, tail)
                part = (acc[0:8] + acc[8:16]) + (acc[16:24] + tail)
                total = part if total is None else total + part
                if h == heads[-1]:
                    is_den = lax.broadcasted_iota(jnp.int32, (8, T), 0) == DH - 24
                    ok = ~is_den | ((low >= DEN_LO) & (high <= DEN_HI))
                    flag[...] = jnp.where(ok & (jnp.abs(total) <= F32_MAX), flag[...], 1.0)
                due(total[:, T - 128:])
                yield
        return gen(), len(heads)

    def weighted_values(h, qb, p_src, paced=False):
        def gen():
            acc = None
            for c in range(S // CK):
                p = jnp.concatenate(
                    [_load_bf16(p_src, (qb, t), c * CK, CK) for t in range(NT)], axis=1)
                a = _dot(_load_bf16(vt, (h, c), 0, HP), p)
                if paced:
                    tap(a)
                acc = a if acc is None else acc + a
                if c == S // CK - 1:
                    for t in range(NT):
                        ot[h, qb, t] = acc[:, _lanes(t)]
                yield
        return gen(), S // CK

    def attention_with_max():
        def body(item, carry):
            h, qb, t = item // (NB * NT), item // NT % NB, item % NT
            q = qt[h, qb, t]

            def scores(c):
                return _dot(kk[h, pl.ds(pl.multiple_of(c * CK, CK), CK), :], q)

            def row_max(c, m):
                return jnp.maximum(m, jnp.max(scores(c), axis=0, keepdims=True))

            m = lax.fori_loop(0, S // CK, row_max, jnp.full((1, 128), -jnp.inf, F32))

            def values(c, acc):
                return acc + _dot(vt[h, c], jnp.exp2(scores(c) - m).astype(BF16))

            ot[h, qb, t] = lax.fori_loop(0, S // CK, values, jnp.zeros((HP, 128), F32))
            return carry
        lax.fori_loop(0, H * NB * NT, body, 0)

    def own_block(emit):
        pl.when(one[0] == 1)(emit)

    def attention(peeled):
        def step(i, kb_cur, p_dst, kb_next, p_src):
            pace_begin()
            _overlap(_chain(*(exp_scores(i + 1, qb, kb_cur, p_dst) for qb in range(NB))),
                     _chain(*(weighted_values(i, qb, p_src) for qb in range(NB))),
                     spread_keys(jnp.minimum(i + 2, H - 1), kb_next))
            pace_end()

        def body(i, carry):
            pl.when(i % 2 == 0)(lambda: step(i, kb_b, p_b, kb_a, p_a))
            pl.when(i % 2 == 1)(lambda: step(i, kb_a, p_a, kb_b, p_b))
            return carry

        if peeled:
            own_block(lambda: step(0, kb_b, p_b, kb_a, p_a))
        lax.fori_loop(int(peeled), H - 1, body, 0)

        pace_begin()
        early, late = range(H - 1), range(H - 1, H)
        for qb in range(NB):
            values = weighted_values(H - 1, qb, p_b, paced=True)
            if qb:
                _overlap(values, _chain(check_block(qb - 1, late), heads_to_rhs(qb - 1)))
            else:
                _overlap(values, _chain(*(check_block(j, early) for j in range(NB))))
        _overlap(check_block(NB - 1, late))
        pace_end()

        @pl.when(jnp.max(flag[...]) > 0.0)
        def _():
            attention_with_max()

            def redo(n, carry):
                pace_begin()
                head_to_rhs(n // H, n % 2, n // 2 % (H // 2))
                return carry
            lax.fori_loop(0, (NB - 1) * H, redo, 0)

    def block_product(lhs, rhs, rows, finish):
        groups = range(0, rows, RG)
        acc = {}
        left = [4, 2, 2, 4]
        for i, targets in _PRODUCT_ORDER:
            m = _dot(lhs(i), rhs(i))
            for blk, _ in targets:
                left[blk] -= 1
            for r in groups:
                piece = m[r:r + RG]
                tap(piece)
                for blk, sign in targets:
                    if (blk, r) not in acc:
                        acc[blk, r] = (piece, sign)
                        continue
                    old, old_sign = acc[blk, r]
                    if old_sign < 0:
                        new = piece - old
                    else:
                        new = old + piece if sign > 0 else old - piece
                    acc[blk, r] = (new, 1)
                    if not left[blk]:
                        finish(blk, r, acc.pop((blk, r))[0])
                yield

    def product_steps(rows):
        return 7 * (rows // RG)

    def moments(load, twice=False):
        total = None
        for n in range(8):
            x = gate(load(n)) if n % 4 == 0 else load(n)
            part = jnp.sum(x.reshape(7, 8, 128), axis=0)
            total = part if total is None else total + part
            if n % 4 == 3:
                due(total)
                yield
        mean = jnp.sum(total, axis=0, keepdims=True) * (1.0 / D)
        squares = total = None
        for n in range(8):
            x = gate(load(n)) if n % 2 == 0 else load(n)
            d = (x - mean).reshape(7, 8, 128)
            part = jnp.sum(d * d, axis=0)
            squares = part if squares is None else squares + part
            if twice:
                part = jnp.sum(d, axis=0)
                total = part if total is None else total + part
            if n % 2 == 1:
                due(squares + total if twice else squares)
                yield
        var = jnp.sum(squares, axis=0, keepdims=True) * (1.0 / D)
        rstd = lax.rsqrt(var + EPS)
        if not twice:
            return mean, rstd
        mean_y = jnp.sum(total, axis=0, keepdims=True) * (1.0 / D) * rstd
        var_y = var * rstd * rstd - mean_y * mean_y
        return mean, rstd, mean_y, lax.rsqrt(var_y + EPS)

    def tile_rows(ref, j, u):
        return lambda n: ref[j, 56 * n:56 * (n + 1), _lanes(u)]

    def norm_to_rhs_gen(src_ref, j):
        for t in range(2):
            stats = []
            for u in (t, t + 2):
                stats.append((yield from moments(tile_rows(src_ref, j, u))))
            for r in range(0, HD, 16):
                blocks = [
                    (gate(src_ref[j, fh * HD + r:fh * HD + r + 16, _lanes(t + 2 * th)])
                     - stats[th][0]) * stats[th][1] for fh, th in quadrants]
                put_rhs(rb.at[j], t, r, *blocks)
                yield

    def norm_to_rhs(src_ref, j):
        return norm_to_rhs_gen(src_ref, j), 2 * (12 + 14)

    def norm_twice(j):
        def gen():
            for t in range(2):
                stats = []
                for u in (t, t + 2):
                    stats.append((yield from moments(tile_rows(xs, j, u), twice=True)))
                for r in range(0, HD, 16):
                    blocks = []
                    for fh, th in quadrants:
                        mean, rstd, mean_y, rstd_y = stats[th]
                        where = (j, slice(fh * HD + r, fh * HD + r + 16), _lanes(t + 2 * th))
                        y = (gate(xs[where]) - mean) * rstd
                        ys[where] = y
                        blocks.append((y - mean_y) * rstd_y)
                    put_rhs(rb.at[j], t, r, *blocks)
                    yield
        return gen(), 2 * (12 + 14)

    def load_x(j):
        def gen():
            for r in range(0, D, 64):
                xs[j, r:r + 64] = io_buf[j, r:r + 64].astype(F32)
                yield
        return _chain((gen(), D // 64), norm_to_rhs(xs, j))

    def qkv(j):
        rhs = rhs_of(rb, j, HD)
        row = lax.broadcasted_iota(jnp.int32, (HP, HT), 0)

        def put_q(h, th, q):
            q = jnp.where(row < DH, q * QSCALE, 0.0)
            qf[h, j, :, th * HT:(th + 1) * HT] = q
            for t in range(2):
                qt[h, j, 2 * th + t] = q[:, _lanes(t)].astype(BF16)

        def put_k(h, th, k):
            k = k.astype(BF16).T
            kk[h, j * T + th * HT:j * T + (th + 1) * HT, :] = k
            if j == 0 and th == 0:
                kn[h] = k[0:NV].astype(F32)

        def put_v(h, th, v):
            v = jnp.where(row < DH, v, (row == DH).astype(F32))
            for t in range(2):
                vt[h, j * NT + 2 * th + t] = v[:, _lanes(t)].astype(BF16)

        def by_head(put):
            pieces = {}

            def finish(blk, r, piece):
                fh, th = quadrants[blk]
                pieces.setdefault(blk, []).append(piece)
                if r + RG == HD:
                    pieces[blk].append(jnp.zeros((8, HT), F32))
                have = sum(p.shape[0] for p in pieces[blk])
                for i in range(H // 2):
                    if r < i * DH + HP <= have:
                        c = jnp.concatenate(pieces[blk], axis=0)
                        put(fh * (H // 2) + i, th, c[i * DH:i * DH + HP])
            return finish

        return [(block_product(lhs_of(aqkv, n * HD, HD), rhs, HD, by_head(put)),
                 product_steps(HD)) for n, put in ((2, put_v), (1, put_k), (0, put_q))]

    def head_to_rhs(j, t, i):
        blocks = [gate(ot[fh * (H // 2) + i, j, t + 2 * th]) for fh, th in quadrants]
        put_rhs(rb.at[j], t, i * HP if isinstance(i, int) else pl.multiple_of(i * HP, HP),
                *(acc * (1.0 / acc[24:32])[DH - 24:DH - 23] for acc in blocks))

    def heads_to_rhs(j):
        def gen():
            for t in range(2):
                for i in range(H // 2):
                    head_to_rhs(j, t, i)
                    yield
        return gen(), H

    def place(blk, r):
        fh, th = quadrants[blk]
        return slice(fh * HD + r, fh * HD + r + RG), slice(th * HT, (th + 1) * HT)

    def proj_o(j):
        def finish(blk, r, c):
            rows, cols = place(blk, r)
            xs[j, rows, cols] = xs[j, rows, cols] + c
        return block_product(lhs_of(ao, 0, HD), rhs_of(rb, j, 256), HD, finish), product_steps(HD)

    def mix1(j):
        def finish(blk, r, c):
            rows, cols = place(blk, r)
            hbuf[rows, HALO + j * T + cols.start:HALO + j * T + cols.stop] = _gelu(c)
        return block_product(lhs_of(a1, 0, HD), rhs_of(rb, j, HD), HD, finish), product_steps(HD)

    def shift_to_rhs(j):
        def shifted(row, u):
            t0 = HALO + j * T + u * 128 - (1, -1, 2, -2)[row // C4]
            return gate(hbuf[row:row + 16, t0:t0 + 128])

        def gen():
            for t in range(2):
                for r in range(0, HD, 16):
                    blocks = [shifted(fh * HD + r, t + 2 * th) for fh, th in quadrants]
                    put_rhs(rb.at[j], t, r, *blocks)
                    yield
        return gen(), 28

    def mix2(j):
        def finish(blk, r, c):
            rows, cols = place(blk, r)
            x1 = ys[j, rows, cols] + c
            ys[j, rows, cols] = x1
            xs[j, rows, cols] = xs[j, rows, cols] + x1
        return block_product(lhs_of(a2, 0, HD), rhs_of(rb, j, HD), HD, finish), product_steps(HD)

    def mlp1(j):
        def gen():
            ready = []

            def activate():
                n, r, blocks = ready.pop(0)
                blocks = [_gelu(c) for c in blocks]
                for t in range(2):
                    put_rhs(gb.at[j % 2], t, n * CN + r, *(c[:, _lanes(t)] for c in blocks))

            for n in range(HF // CN):
                got = {}

                def finish(blk, r, c, n=n, got=got):
                    got[blk, r] = c
                    if all((b, r) in got for b in range(4)):
                        ready.append((n, r, [got.pop((b, r)) for b in range(4)]))

                waiting = len(ready)
                for x, _ in enumerate(block_product(
                        lhs_of(a3, n * CN, CN), rhs_of(rb, j, HD), CN, finish)):
                    if waiting and x % 7 == 3:
                        activate()
                        waiting -= 1
                    yield
            while ready:
                activate()
        return gen(), product_steps(HF)

    def mlp2(j, last=False):
        def finish(blk, r, c):
            rows, cols = place(blk, r)
            x = xs[j, rows, cols] + c
            if last:
                io_buf[j, rows, cols] = x.astype(BF16)
                if j == NB - 1 and r + RG == HD:
                    out_part_copy(blk).start()
            else:
                xs[j, rows, cols] = x

        def gen():
            yield from block_product(lhs_of(a4, 0, HD), rhs_of(gb, j % 2, HF), HD, finish)
            if last and j < NB - 1:
                out_copy(j).start()
        return gen(), product_steps(HD)

    def start_attention(nv, *extra):
        def emit():
            pace_begin()
            _overlap(_chain(*(exp_scores(0, qb, kb_a, p_a, nv) for qb in range(NB))),
                     spread_keys(1, kb_b), *(make() for make in extra))
            pace_end()
        pace_end()
        own_block(emit)

    def into_first_layer():
        x_copy(0).start()
        wv_copy.start()
        x_copy(1).start()
        flag[...] = jnp.zeros((8, T), F32)
        one[0] = 1
        hbuf[:, 0:HALO] = jnp.zeros((D, HALO), F32)
        hbuf[:, HALO + S:] = jnp.zeros((D, HALO), F32)
        pace_begin()
        wq, wk, wv = (prep(aqkv, n * HD, rows_of(wqkv_raw), n * D, D) for n in range(3))
        v, k, q = zip(*(qkv(j) for j in range(NB)))
        x_copy(0).wait()
        wv_copy.wait()
        wqk_copy.start()
        _overlap(load_x(0), wv)
        x_copy(1).wait()
        x_copy(2).start()
        x_copy(3).start()
        _overlap(v[0], load_x(1))
        wqk_copy.wait()
        _overlap(v[1], _chain(wk, wq))
        x_copy(2).wait()
        x_copy(3).wait()
        for c in w_copies:
            c.start()
        _overlap(_chain(k[0], q[0]), load_x(2))
        _overlap(_chain(k[1], q[1]), load_x(3))
        _overlap(_chain(k[2], q[2], v[2]), spread_keys(0, kb_a))
        for c in w_copies:
            c.wait()
        _overlap(_chain(k[3], q[3], v[3]), _ahead(_chain(
            prep(ao, 0, head_rows_of(wo_raw), 0, D), prep(a1, 0, rows_of(w1_raw), 0, D),
            prep(a2, 0, rows_of(w2_raw), 0, D), prep_w4())))
        start_attention(160, lambda: _ahead(prep(a3, 0, rows_of(w3_raw), 0, F)))

    def after_attention(last):
        pace_begin()
        _overlap(proj_o(0), heads_to_rhs(3))
        _overlap(_chain(proj_o(1), proj_o(2), proj_o(3), mix1(0), mix1(1), mix1(2)),
                 _chain(norm_twice(0), norm_twice(1), norm_twice(2), norm_twice(3),
                        shift_to_rhs(0)))
        _overlap(mix2(0), shift_to_rhs(1))
        _overlap(mix2(1), norm_to_rhs(ys, 0))
        _overlap(mix1(3))
        _overlap(mlp1(0), _chain(norm_to_rhs(ys, 1), shift_to_rhs(2), shift_to_rhs(3)))
        _overlap(mlp2(0, last))
        _overlap(mix2(2))
        _overlap(mlp1(1), norm_to_rhs(ys, 2))
        _overlap(mix2(3))

    def into_second_layer():
        v, k, q = zip(*(qkv(j) for j in range(NB)))
        _overlap(mlp2(1), _chain(norm_to_rhs(ys, 3), norm_to_rhs(xs, 0)))
        _overlap(mlp1(2))
        _overlap(_chain(k[0], q[0], v[0]), norm_to_rhs(xs, 1))
        _overlap(mlp2(2), spread_keys(0, kb_a))
        _overlap(mlp1(3))
        _overlap(_chain(k[1], q[1], v[1]), norm_to_rhs(xs, 2))
        _overlap(mlp2(3))
        _overlap(_chain(k[2], q[2], v[2]), norm_to_rhs(xs, 3))
        _overlap(_chain(k[3], q[3], v[3]))
        start_attention(192)

    def into_output():
        _overlap(mlp2(1, True), norm_to_rhs(ys, 3))
        _overlap(mlp1(2))
        _overlap(mlp1(3))
        _overlap(mlp2(2, True))
        _overlap(mlp2(3, True))
        pace_end()
        for j in range(NB - 1):
            out_copy(j).wait()
        for blk in range(4):
            out_part_copy(blk).wait()

    into_first_layer()
    attention(peeled=True)
    after_attention(last=False)
    into_second_layer()
    attention(peeled=False)
    after_attention(last=True)
    into_output()


@jax.jit
def pallas_interleave_layers__mha_block__mixer_s_mlp__prompt_kernel(
    A_x: jax.Array,
    A_wqkv: jax.Array,
    A_wo: jax.Array,
    B_x: jax.Array,
    B_w1: jax.Array,
    B_w2: jax.Array,
    B_w3: jax.Array,
    B_w4: jax.Array,
):
    del B_x
    vm = pltpu.VMEM
    scratch = [
        vm((32, 128), F32),
        vm((DH, NV, 128), F32),
        vm((DH, NV, 128), F32),
        vm((NB, NT, S, 128), BF16),
        vm((NB, NT, S, 128), BF16),
        vm((8, T), F32),
        vm((NB, 7, 2, 256, 128), BF16),
        vm((NB, D, T), F32),
        vm((NB, D, T), F32),
        vm((2, 7, 2, HF, 128), BF16),
        vm((7, 2, 768, 128), BF16),
        vm((7, 2, 256, 128), BF16),
        vm((7, 2, 256, 128), BF16),
        vm((7, 2, 256, 128), BF16),
        vm((7, 2, HF, 128), BF16),
        vm((7, HF // 128, 256, 128), BF16),
        vm((D, S + 2 * HALO), F32),
        vm((H, NB, NT, HP, 128), F32),
        vm((H, NB, NT, HP, 128), BF16),
        vm((H, NB, HP, T), F32),
        vm((H, S, HP), BF16),
        vm((H, NV, HP), F32),
        vm((H, S // CK, HP, CK), BF16),
        vm((NB, D, T), BF16),
        vm((512, 3 * D), BF16), vm((D, D), BF16), vm((D, D), BF16), vm((D, D), BF16),
        vm((512, F), BF16), vm((512, F), BF16),
        pltpu.SMEM((1,), jnp.int32),
        pltpu.SemaphoreType.DMA((NB + 7,)),
        pltpu.SemaphoreType.DMA((NB + 3,)),
    ]
    hbm = pl.BlockSpec(memory_space=pl.ANY)
    out = pl.pallas_call(
        _kernel,
        in_specs=[hbm] * 7,
        out_specs=hbm,
        out_shape=jax.ShapeDtypeStruct((D, S), BF16),
        scratch_shapes=scratch,
        compiler_params=pltpu.CompilerParams(vmem_limit_bytes=120 * 2**20),
    )(A_x[0].T, A_wqkv, A_wo, B_w1, B_w2, B_w3, B_w4.T)
    return out.T[None]
```
